```python
import os as _os
_os.environ.setdefault("JAX_PLATFORMS", "cpu")
import jax
import jax.numpy as jnp

def _softmax(x, axis=-1):
    return jax.nn.softmax(x, axis=axis)
def _gelu(x):
    return jax.nn.gelu(x, approximate=True)
def _silu(x):
    return jax.nn.silu(x)
def _sigmoid(x):
    return jax.nn.sigmoid(x)
def _layernorm(x, axis=-1, eps=1e-5):
    m = jnp.mean(x, axis=axis, keepdims=True)
    v = jnp.var(x, axis=axis, keepdims=True)
    return (x - m) / jnp.sqrt(v + eps)
def _scatter_add(tgt, idx, src, axis=0):
    return tgt.at[idx].add(src)
def _segment_sum(src, seg, n):
    return jax.ops.segment_sum(src, seg, n)
class _Rng:
    def __init__(self, key):
        self._k = key
    def _next(self):
        self._k, sub = jax.random.split(self._k)
        return sub
    def normal(self, shape):
        return jax.random.normal(self._next(), shape, dtype=jnp.bfloat16)
    def randint(self, lo, hi, shape):
        return jax.random.randint(self._next(), shape, lo, hi, dtype=jnp.int32)
    def uniform(self, shape, lo=0.0, hi=1.0):
        return jax.random.uniform(self._next(), shape, jnp.bfloat16, lo, hi)
    def permutation(self, n):
        return jax.random.permutation(self._next(), n)


kernel_name = 'gated_mix__grouped_kv_mqa__glu_gated_reglu__prompt'

def setup_inputs():
    _rng = _Rng(jax.random.key(int.from_bytes(__import__("os").urandom(4), "little")))
    _w = (lambda a: (lambda t: t.astype(jnp.bfloat16) if jnp.issubdtype(t.dtype, jnp.floating) else t)(jnp.asarray(a)))
    def _A_setup():
        B, S, D, H = 1, 2048, 640, 32
        Dh = D // H
        return {
            "x": _w((lambda *s: _rng.normal(s) * 0.05)(B, S, D)),
            "wq": _w((lambda *s: _rng.normal(s) * 0.2)(D, H * Dh)),
            "wk": _w((lambda *s: _rng.normal(s) * 0.2)(D, Dh)),
            "wv": _w((lambda *s: _rng.normal(s) * 0.05)(D, Dh)),
            "wo": _w((lambda *s: _rng.normal(s) * 0.05)(H * Dh, D)),
        }
    _A_in = _A_setup()

    def _B_setup():
        B, S, D, F = 1, 2048, 640, 1536
        return {
            "x": _w((lambda *s: _rng.normal(s) * 0.05)(B, S, D)),
            "W_gate": _w((lambda *s: _rng.normal(s) * 0.4)(D, F) * (2.0 / D) ** 0.5),
            "W_up": _w((lambda *s: _rng.normal(s) * 0.4)(D, F) * (2.0 / D) ** 0.5),
            "W_down": _w((lambda *s: _rng.normal(s) * 0.4)(F, D) * (1.0 / F) ** 0.5),
        }
    _B_in = _B_setup()

    return {
        "A_x": _A_in["x"],
        "A_wq": _A_in["wq"],
        "A_wk": _A_in["wk"],
        "A_wv": _A_in["wv"],
        "A_wo": _A_in["wo"],
        "B_x": _B_in["x"],
        "B_W_gate": _B_in["W_gate"],
        "B_W_up": _B_in["W_up"],
        "B_W_down": _B_in["W_down"],
        "gate_w": _w((lambda *s: _rng.normal(s) * 0.05)(640) * 16.0),
    }

def reference(A_x, A_wq, A_wk, A_wv, A_wo, B_x, B_W_gate, B_W_up, B_W_down, gate_w):
    def _A_ref(x, wq, wk, wv, wo):
        B, S, D = x.shape
        H = 32
        Dh = D // H
        q = (lambda x, *d: x.transpose(*d))((x @ wq).reshape(B, S, H, Dh), 0, 2, 1, 3)
        k = x @ wk
        v = x @ wv
        scores = jnp.einsum("bhqd,bkd->bhqk", q, k) * (Dh ** -0.5)
        p = _softmax(scores, axis=-1)
        o = jnp.einsum("bhqk,bkd->bhqd", p, v)
        return (lambda x, *d: x.transpose(*d))(o, 0, 2, 1, 3).reshape(B, S, H * Dh) @ wo

    def _B_ref(x, W_gate, W_up, W_down):
        gate = jnp.einsum("bsd,df->bsf", x, W_gate)
        up = jnp.einsum("bsd,df->bsf", x, W_up)
        gate = gate * (lambda x, dt: x.astype(dt))(gate > 0, gate.dtype)
        h = gate * up
        return jnp.einsum("bsf,fd->bsd", h, W_down)

    x = A_x
    g = _sigmoid((x * gate_w).sum(-1, keepdims=True))
    a = _A_ref(x, A_wq, A_wk, A_wv, A_wo)
    b = _B_ref(x, B_W_gate, B_W_up, B_W_down)
    return g * a + (1 - g) * b
```

```python
import functools
import math

import jax
import jax.numpy as jnp
import jax.experimental.pallas as pl
import jax.experimental.pallas.tpu as pltpu

F32 = jnp.float32
BF16 = jnp.bfloat16
U32 = jnp.uint32

S = 2048
D = 640
H = 32
DH = 20
FF = 1536
HPG = 6
NG = 6
VROWS = 24
TQ = 512
CK = 256
FC = 512
LOG2E = 1.4426950408889634


def _pack(x_bf16):
    return pltpu.bitcast(x_bf16, U32)


def _unpack(x_u32):
    return pltpu.bitcast(x_u32, BF16)


def _kernel(x_ref, wq_ref, wk_ref, wv_ref, wo_ref, gw_ref, wg_hbm, wu_hbm, wd_hbm,
            o_ref,
            kp_ref, vt_ref, wqt_ref, wop_ref, qt_ref, sa_ref, sb_ref, ma_ref, mb_ref,
            ot_ref, wg_ref, wu_ref, wd_ref, sems):
    step = pl.program_id(0)

    def weight_copies():
        return (pltpu.make_async_copy(wg_hbm, wg_ref, sems.at[0]),
                pltpu.make_async_copy(wu_hbm, wu_ref, sems.at[1]),
                pltpu.make_async_copy(wd_hbm, wd_ref, sems.at[2]))

    @pl.when(step == 0)
    def _setup():
        for cp in weight_copies():
            cp.start()
        x = x_ref[...]
        wk = wk_ref[...]
        wk_rep = jnp.concatenate([wk] * HPG + [jnp.zeros((D, 128 - HPG * DH), BF16)], axis=1)
        krep = jnp.dot(x, wk_rep, preferred_element_type=F32) * (DH ** -0.5 * LOG2E)
        lane = jax.lax.broadcasted_iota(jnp.int32, (S, 128), 1)
        for j in range(HPG):
            m = (lane >= j * DH) & (lane < (j + 1) * DH)
            kp_ref[j] = _pack(jnp.where(m, krep, 0.0).astype(BF16))
        wv = wv_ref[...]
        wv_pad = jnp.concatenate([wv, jnp.zeros((D, VROWS - DH), BF16)], axis=1)
        vt = jax.lax.dot_general(wv_pad, x, (((0,), (1,)), ((), ())),
                                 preferred_element_type=F32)
        row = jax.lax.broadcasted_iota(jnp.int32, (VROWS, S), 0)
        vt = vt.astype(BF16).astype(F32)
        vt_ref[...] = jnp.where(row == DH, 1.0, vt)
        wqt = wq_ref[...].astype(F32).T
        for g in range(NG):
            n = min(HPG, H - g * HPG) * DH
            blk = jnp.concatenate(
                [wqt[g * HPG * DH: g * HPG * DH + n], jnp.zeros((128 - n, D), F32)], axis=0)
            wqt_ref[g] = _pack(blk.astype(BF16))
        wo = wo_ref[...].astype(F32)
        for hp in range(H // 2):
            blk = jnp.concatenate(
                [wo[2 * hp * DH: (2 * hp + 1) * DH], jnp.zeros((VROWS - DH, D), F32),
                 wo[(2 * hp + 1) * DH: (2 * hp + 2) * DH], jnp.zeros((VROWS - DH, D), F32)],
                axis=0)
            wop_ref[pl.ds(hp * VROWS, VROWS), :] = _pack(blk.astype(BF16))

    row0 = pl.multiple_of(step * TQ, TQ)
    xb = x_ref[pl.ds(row0, TQ), :]

    for g in range(NG):
        qt = jax.lax.dot_general(_unpack(wqt_ref[g]), xb, (((1,), (1,)), ((), ())),
                                 preferred_element_type=F32)
        qt_ref[g] = _pack(qt.astype(BF16))

    def qk_chunk(j, q, c, s_ref, mpart):
        kc = _unpack(kp_ref[j, pl.ds(c * CK // 2, CK // 2), :])
        s = jnp.dot(kc, q, preferred_element_type=F32)
        s_ref[pl.ds(c * CK, CK), :] = s
        return jnp.maximum(mpart, jnp.max(s.reshape(CK // 8, 8, TQ), axis=0))

    def pv_chunk(c, s_cur, m_c, acc):
        p = jnp.exp2(s_cur[pl.ds(c * CK, CK), :] - m_c).astype(BF16)
        vc = vt_ref[:, pl.ds(c * CK, CK)]
        return acc + jnp.dot(vc, p, preferred_element_type=F32)

    def finish_head(h, acc):
        inv = 1.0 / acc[DH:DH + 1, :]
        ot_ref[h] = acc * inv

    def attn_step(h_next, h_cur, s_next, s_cur, m_next, m_cur):
        g = h_next // HPG
        j = h_next % HPG
        q = _unpack(qt_ref[g])
        m_c = m_cur[...]
        acc = jnp.zeros((VROWS, TQ), F32)
        mpart = jnp.full((8, TQ), -jnp.inf, F32)
        for c in range(S // CK):
            mpart = qk_chunk(j, q, c, s_next, mpart)
            acc = pv_chunk(c, s_cur, m_c, acc)
        m_next[...] = jnp.max(mpart, axis=0, keepdims=True)
        finish_head(h_cur, acc)

    q0 = _unpack(qt_ref[0])
    mpart = jnp.full((8, TQ), -jnp.inf, F32)
    for c in range(S // CK):
        mpart = qk_chunk(0, q0, c, sa_ref, mpart)
    ma_ref[...] = jnp.max(mpart, axis=0, keepdims=True)

    def body(i, carry):
        h = 2 * i
        attn_step(h + 1, h, sb_ref, sa_ref, mb_ref, ma_ref)
        attn_step(h + 2, h + 1, sa_ref, sb_ref, ma_ref, mb_ref)
        return carry

    jax.lax.fori_loop(0, H // 2 - 1, body, 0)
    attn_step(H - 1, H - 2, sb_ref, sa_ref, mb_ref, ma_ref)

    @pl.when(step == 0)
    def _wait_weights():
        for cp in weight_copies():
            cp.wait()

    m_c = mb_ref[...]
    acc = jnp.zeros((VROWS, TQ), F32)
    for c in range(S // CK):
        acc = pv_chunk(c, sb_ref, m_c, acc)
    finish_head(H - 1, acc)

    b = jnp.zeros((TQ, D), F32)
    for f in range(FF // FC):
        gate = jnp.dot(xb, wg_ref[:, pl.ds(f * FC, FC)], preferred_element_type=F32)
        up = jnp.dot(xb, wu_ref[:, pl.ds(f * FC, FC)], preferred_element_type=F32)
        hh = (jnp.maximum(gate, 0.0) * up).astype(BF16)
        b = b + jnp.dot(hh, wd_ref[pl.ds(f * FC, FC), :], preferred_element_type=F32)

    ot = ot_ref[...].reshape(H * VROWS, TQ).astype(BF16)
    a = jax.lax.dot_general(ot, _unpack(wop_ref[...]), (((0,), (0,)), ((), ())),
                            preferred_element_type=F32)

    z = jnp.sum(xb.astype(F32) * gw_ref[...].astype(F32), axis=-1, keepdims=True)
    g = 1.0 / (1.0 + jnp.exp(-z))
    o_ref[...] = (g * a + (1.0 - g) * b).astype(o_ref.dtype)


@jax.jit
def pallas_gated_mix__grouped_kv_mqa__glu_gated_reglu__prompt_kernel(
    A_x: jax.Array,
    A_wq: jax.Array,
    A_wk: jax.Array,
    A_wv: jax.Array,
    A_wo: jax.Array,
    B_x: jax.Array,
    B_W_gate: jax.Array,
    B_W_up: jax.Array,
    B_W_down: jax.Array,
    gate_w: jax.Array,
):
    x = A_x.reshape(S, D)
    gw = gate_w.reshape(1, D)

    def full(shape):
        return pl.BlockSpec(shape, lambda i: (0,) * len(shape))

    any_spec = pl.BlockSpec(memory_space=pl.ANY)
    out = pl.pallas_call(
        _kernel,
        grid=(S // TQ,),
        in_specs=[full((S, D)), full((D, D)), full((D, DH)), full((D, DH)), full((D, D)),
                  full((1, D)), any_spec, any_spec, any_spec],
        out_specs=pl.BlockSpec((TQ, D), lambda i: (i, 0)),
        out_shape=jax.ShapeDtypeStruct((S, D), BF16),
        scratch_shapes=[
            pltpu.VMEM((HPG, S // 2, 128), U32),
            pltpu.VMEM((VROWS, S), F32),
            pltpu.VMEM((NG, 64, D), U32),
            pltpu.VMEM((H * VROWS // 2, D), U32),
            pltpu.VMEM((NG, 64, TQ), U32),
            pltpu.VMEM((S, TQ), F32),
            pltpu.VMEM((S, TQ), F32),
            pltpu.VMEM((1, TQ), F32),
            pltpu.VMEM((1, TQ), F32),
            pltpu.VMEM((H, VROWS, TQ), F32),
            pltpu.VMEM((D, FF), BF16),
            pltpu.VMEM((D, FF), BF16),
            pltpu.VMEM((FF, D), BF16),
            pltpu.SemaphoreType.DMA((3,)),
        ],
        compiler_params=pltpu.CompilerParams(
            dimension_semantics=("arbitrary",),
            vmem_limit_bytes=100 * 1024 * 1024,
        ),
    )(x, A_wq, A_wk, A_wv, A_wo, gw, B_W_gate, B_W_up, B_W_down)
    return out.reshape(1, S, D)
```

```python
import functools
import math

import jax
import jax.numpy as jnp
import jax.experimental.pallas as pl
import jax.experimental.pallas.tpu as pltpu

F32 = jnp.float32
BF16 = jnp.bfloat16
U32 = jnp.uint32

S = 2048
D = 640
H = 32
DH = 20
FF = 1536
HPG = 6
NG = 6
BROW = HPG * DH
VROWS = 24
TQ = 512
CK = 128
NCK = S // CK
LA = 2
NBUF = LA + 1
FC = 512
LOG2E = 1.4426950408889634
SHIFT_MAX = 32.0
VMIN = 2.0 ** -30


def _pack(x_bf16):
    return pltpu.bitcast(x_bf16, U32)


def _unpack(x_u32):
    return pltpu.bitcast(x_u32, BF16)


def _pk16(e):
    n, w = e.shape
    e4 = e.reshape(n // 16, 2, 8, w)
    return pltpu.pack_elementwise([e4[:, 0], e4[:, 1]], packed_dtype=BF16).reshape(n // 2, w)


def _kernel(x_ref, wq_ref, wkt_ref, wvt_ref, gw_ref, wo_hbm, wg_hbm, wu_hbm, wd_hbm,
            o_ref,
            kf_ref, kp_ref, vt_ref, wqt_ref, wop_ref, qt_ref, p_ref, s_ref,
            ot_ref, wo_ref, wg_ref, wu_ref, wd_ref, stat_ref, sems):
    step = pl.program_id(0)

    def weight_copies():
        return (pltpu.make_async_copy(wo_hbm, wo_ref, sems.at[0]),
                pltpu.make_async_copy(wg_hbm, wg_ref, sems.at[1]),
                pltpu.make_async_copy(wu_hbm, wu_ref, sems.at[2]),
                pltpu.make_async_copy(wd_hbm, wd_ref, sems.at[3]))

    @pl.when(step == 0)
    def _setup():
        for cp in weight_copies():
            cp.start()
        x = x_ref[...]
        wkt = wkt_ref[...].astype(F32)
        wkt_rep = jnp.concatenate([wkt] * HPG + [jnp.zeros((128 - BROW, D), F32)], axis=0)
        krep = jax.lax.dot_general(x, wkt_rep.astype(BF16), (((1,), (1,)), ((), ())),
                                   preferred_element_type=F32) * (DH ** -0.5 * LOG2E)
        krep = krep.astype(BF16).astype(F32)
        kf_ref[...] = krep
        k2 = jnp.sum(krep * krep, axis=1, keepdims=True) * (1.0 / HPG)
        stat_ref[0] = jnp.max(k2)
        ev = kf_ref[pl.ds(0, S // 2, stride=2), :].reshape(S // 16, 1, 8, 128)
        od = kf_ref[pl.ds(1, S // 2, stride=2), :].reshape(S // 16, 1, 8, 128)
        kperm = jnp.concatenate([ev, od], axis=1).reshape(S, 128)
        lane = jax.lax.broadcasted_iota(jnp.int32, (S, 128), 1)
        for j in range(HPG):
            m = (lane >= j * DH) & (lane < (j + 1) * DH)
            kj = jnp.where(m, kperm, jnp.where(lane == BROW, 1.0, 0.0))
            kp_ref[j] = _pack(kj.astype(BF16))
        wvt = wvt_ref[...].astype(F32)
        wvt_pad = jnp.concatenate([wvt, jnp.zeros((VROWS - DH, D), F32)], axis=0)
        vt = jax.lax.dot_general(wvt_pad, x, (((1,), (1,)), ((), ())),
                                 preferred_element_type=F32)
        vt = vt.astype(BF16).astype(F32)
        stat_ref[1] = jnp.max(jnp.abs(vt))
        row = jax.lax.broadcasted_iota(jnp.int32, (VROWS, S), 0)
        vt_ref[...] = jnp.where(row == DH, 1.0, vt)
        wqt = wq_ref[...].astype(F32).T
        for g in range(NG):
            n = min(HPG, H - g * HPG) * DH
            blk = jnp.concatenate(
                [wqt[g * BROW: g * BROW + n], jnp.zeros((128 - n, D), F32)], axis=0)
            wqt_ref[g] = _pack(blk.astype(BF16))

    row0 = pl.multiple_of(step * TQ, TQ)
    xb = x_ref[pl.ds(row0, TQ), :]

    kmax2 = stat_ref[0]
    qts, shifts = [], []
    for g in range(NG):
        qt = jax.lax.dot_general(_unpack(wqt_ref[g]), xb, (((1,), (1,)), ((), ())),
                                 preferred_element_type=F32)
        n2 = jnp.sum(qt * qt, axis=0, keepdims=True)
        qts.append(qt)
        shifts.append(jnp.sqrt(n2 * kmax2) * 1.02)
    cmax = shifts[0]
    for c in shifts[1:]:
        cmax = jnp.maximum(cmax, c)
    safe = jnp.logical_and(jnp.max(cmax) <= SHIFT_MAX, stat_ref[1] >= VMIN)
    rowi = jax.lax.broadcasted_iota(jnp.int32, (128, TQ), 0)
    for g in range(NG):
        c = jnp.where(safe, shifts[g], 0.0)
        qt_ref[g] = _pack(jnp.where(rowi == BROW, -c, qts[g]).astype(BF16))

    def scores(g, j, c, n):
        kc = _unpack(kp_ref[j, pl.ds(c * n // 2, n // 2), :])
        return jnp.dot(kc, _unpack(qt_ref[g]), preferred_element_type=F32)

    def finish_head(h, acc):
        inv = 1.0 / acc[DH:DH + 1, :]
        ot_ref[h] = acc * inv

    @pl.when(safe)
    def _fast():
        def produce(g, j, c, slot):
            p_ref[slot] = _pk16(jnp.exp2(scores(g, j, c, CK)))

        def consume(c, slot, acc):
            return acc + jnp.dot(vt_ref[:, pl.ds(c * CK, CK)], _unpack(p_ref[slot]),
                                 preferred_element_type=F32)

        def group(g, nheads, g_next):
            t = 0
            for j in range(nheads):
                acc = jnp.zeros((VROWS, TQ), F32)
                for c in range(NCK):
                    cn = c + LA
                    slot = (t + LA) % NBUF
                    if cn < NCK:
                        produce(g, j, cn, slot)
                    elif j + 1 < nheads:
                        produce(g, j + 1, cn - NCK, slot)
                    elif g_next is not None:
                        produce(g_next, 0, cn - NCK, slot)
                    acc = consume(c, t % NBUF, acc)
                    t += 1
                finish_head(g * HPG + j, acc)

        for c in range(LA):
            produce(0, 0, c, c % NBUF)

        def body(g, carry):
            group(g, HPG, g + 1)
            return carry

        jax.lax.fori_loop(0, NG - 1, body, 0)
        group(NG - 1, H - (NG - 1) * HPG, None)

    @pl.when(jnp.logical_not(safe))
    def _slow():
        def body(h, carry):
            g = h // HPG
            j = h % HPG
            s_ref[...] = scores(g, j, 0, S)
            m = jnp.max(s_ref[...], axis=0, keepdims=True)
            p = _unpack(_pk16(jnp.exp2(s_ref[...] - m)))
            finish_head(h, jnp.dot(vt_ref[...], p, preferred_element_type=F32))
            return carry

        jax.lax.fori_loop(0, H, body, 0)

    @pl.when(step == 0)
    def _wait_weights():
        for cp in weight_copies():
            cp.wait()
        wo = wo_ref[...].astype(F32)
        for hp in range(H // 2):
            blk = jnp.concatenate(
                [wo[2 * hp * DH: (2 * hp + 1) * DH], jnp.zeros((VROWS - DH, D), F32),
                 wo[(2 * hp + 1) * DH: (2 * hp + 2) * DH], jnp.zeros((VROWS - DH, D), F32)],
                axis=0)
            wop_ref[pl.ds(hp * VROWS, VROWS), :] = _pack(blk.astype(BF16))

    b = jnp.zeros((TQ, D), F32)
    for f in range(FF // FC):
        gate = jnp.dot(xb, wg_ref[:, pl.ds(f * FC, FC)], preferred_element_type=F32)
        up = jnp.dot(xb, wu_ref[:, pl.ds(f * FC, FC)], preferred_element_type=F32)
        hh = (jnp.maximum(gate, 0.0) * up).astype(BF16)
        b = b + jnp.dot(hh, wd_ref[pl.ds(f * FC, FC), :], preferred_element_type=F32)

    ot = ot_ref[...].reshape(H * VROWS, TQ).astype(BF16)
    a = jax.lax.dot_general(ot, _unpack(wop_ref[...]), (((0,), (0,)), ((), ())),
                            preferred_element_type=F32)

    z = jnp.sum(xb.astype(F32) * gw_ref[...].astype(F32), axis=-1, keepdims=True)
    g = 1.0 / (1.0 + jnp.exp(-z))
    o_ref[...] = (g * a + (1.0 - g) * b).astype(o_ref.dtype)


@jax.jit
def pallas_gated_mix__grouped_kv_mqa__glu_gated_reglu__prompt_kernel(
    A_x: jax.Array,
    A_wq: jax.Array,
    A_wk: jax.Array,
    A_wv: jax.Array,
    A_wo: jax.Array,
    B_x: jax.Array,
    B_W_gate: jax.Array,
    B_W_up: jax.Array,
    B_W_down: jax.Array,
    gate_w: jax.Array,
):
    x = A_x.reshape(S, D)
    gw = gate_w.reshape(1, D)

    def full(shape):
        return pl.BlockSpec(shape, lambda i: (0,) * len(shape))

    any_spec = pl.BlockSpec(memory_space=pl.ANY)
    out = pl.pallas_call(
        _kernel,
        grid=(S // TQ,),
        in_specs=[full((S, D)), full((D, D)), full((DH, D)), full((DH, D)),
                  full((1, D)), any_spec, any_spec, any_spec, any_spec],
        out_specs=pl.BlockSpec((TQ, D), lambda i: (i, 0)),
        out_shape=jax.ShapeDtypeStruct((S, D), BF16),
        scratch_shapes=[
            pltpu.VMEM((S, 128), F32),
            pltpu.VMEM((HPG, S // 2, 128), U32),
            pltpu.VMEM((VROWS, S), F32),
            pltpu.VMEM((NG, 64, D), U32),
            pltpu.VMEM((H * VROWS // 2, D), U32),
            pltpu.VMEM((NG, 64, TQ), U32),
            pltpu.VMEM((NBUF, CK // 2, TQ), U32),
            pltpu.VMEM((S, TQ), F32),
            pltpu.VMEM((H, VROWS, TQ), F32),
            pltpu.VMEM((D, D), BF16),
            pltpu.VMEM((D, FF), BF16),
            pltpu.VMEM((D, FF), BF16),
            pltpu.VMEM((FF, D), BF16),
            pltpu.SMEM((2,), F32),
            pltpu.SemaphoreType.DMA((4,)),
        ],
        compiler_params=pltpu.CompilerParams(
            dimension_semantics=("arbitrary",),
            vmem_limit_bytes=100 * 1024 * 1024,
        ),
    )(x, A_wq, A_wk.T, A_wv.T, gw, A_wo, B_W_gate, B_W_up, B_W_down)
    return out.reshape(1, S, D)
```

```python
import jax
import jax.numpy as jnp
import jax.experimental.pallas as pl
import jax.experimental.pallas.tpu as pltpu

F32 = jnp.float32
BF16 = jnp.bfloat16
U32 = jnp.uint32

S = 2048
D = 640
H = 32
DH = 20
FF = 1536
HPG = 6
NG = 6
BROW = HPG * DH
VROWS = 24
TQ = 512
NQB = S // TQ
CK = 128
NCK = S // CK
LA = 2
NBUF = LA + 1
FC = 512
NV = 16
LV = 1
NBV = LV + 1
NVB = TQ // CK * NV
LOG2E = 1.4426950408889634
SHIFT_MAX = 32.0
VMIN = 2.0 ** -30

NT = (((1,), (1,)), ((), ()))
TN = (((0,), (0,)), ((), ()))


def _pack(x_bf16):
    return pltpu.bitcast(x_bf16, U32)


def _unpack(x_u32):
    return pltpu.bitcast(x_u32, BF16)


def _pk16(e):
    n, w = e.shape
    e4 = e.reshape(n // 16, 2, 8, w)
    return pltpu.pack_elementwise([e4[:, 0], e4[:, 1]], packed_dtype=BF16).reshape(n // 2, w)


def _kernel(x_hbm, wq_hbm, wkt_hbm, wvt_hbm, gw_hbm, wo_hbm, wg_hbm, wu_hbm, wd_hbm,
            o_ref,
            x_ref, wq_ref, wo_ref, wg_ref, wu_ref, wd_ref,
            wqt_ref, kf_ref, kp_ref, kb_ref, vt_ref, qt_ref, qf_ref, qb_ref, p_ref, pv_ref,
            s_ref, ot_ref, n2_ref, wkt_ref, wvt_ref, gw_ref, flag_ref, sems):
    step = pl.program_id(0)

    def x_copy(i):
        rows = pl.ds(pl.multiple_of(i * TQ, TQ), TQ)
        return pltpu.make_async_copy(x_hbm.at[rows, :], x_ref.at[rows, :], sems.at[i])

    wk_copy = pltpu.make_async_copy(wkt_hbm, wkt_ref, sems.at[NQB])
    wv_copy = pltpu.make_async_copy(wvt_hbm, wvt_ref, sems.at[NQB + 1])
    wq_copy = pltpu.make_async_copy(wq_hbm, wq_ref, sems.at[NQB + 2])
    late_copies = (pltpu.make_async_copy(wo_hbm, wo_ref, sems.at[NQB + 3]),
                   pltpu.make_async_copy(wg_hbm, wg_ref, sems.at[NQB + 4]),
                   pltpu.make_async_copy(wu_hbm, wu_ref, sems.at[NQB + 5]),
                   pltpu.make_async_copy(wd_hbm, wd_ref, sems.at[NQB + 6]),
                   pltpu.make_async_copy(gw_hbm, gw_ref.at[:, pl.ds(0, D)], sems.at[NQB + 7]))

    def build_qb(qb):
        for g in range(NG):
            n = min(HPG, H - g * HPG) * DH
            for r in list(range(n)) + [BROW]:
                qb_ref[g, r] = jnp.broadcast_to(qf_ref[qb, g, pl.ds(r, 1), :], (8, TQ))

    @pl.when(step == 0)
    def _setup():
        wk_copy.start()
        wv_copy.start()
        wq_copy.start()
        for i in range(NQB):
            x_copy(i).start()

        wq_copy.wait()
        wqt_ref[...] = _pack(wq_ref[...].astype(F32).T.astype(BF16))
        wk_copy.wait()
        wv_copy.wait()
        wkt = wkt_ref[...].astype(F32)
        wkt_rep = jnp.concatenate([wkt] * HPG + [jnp.zeros((128 - BROW, D), F32)],
                                  axis=0).astype(BF16)
        wvt_pad = jnp.concatenate([wvt_ref[...].astype(F32), jnp.zeros((VROWS - DH, D), F32)],
                                  axis=0)

        def chunk(i, carry):
            kmax2, vmax = carry
            x_copy(i).wait()
            rows = pl.ds(pl.multiple_of(i * TQ, TQ), TQ)
            xi = x_ref[rows, :]
            lane = jax.lax.broadcasted_iota(jnp.int32, (TQ, 128), 1)
            vrow = jax.lax.broadcasted_iota(jnp.int32, (VROWS, TQ), 0)
            krep = jax.lax.dot_general(xi, wkt_rep, NT,
                                       preferred_element_type=F32) * (DH ** -0.5 * LOG2E)
            krep = krep.astype(BF16).astype(F32)
            kf_ref[...] = krep
            k2 = jnp.sum(krep * krep, axis=1, keepdims=True)
            kmax2 = jnp.maximum(kmax2, jnp.max(k2.reshape(TQ // 8, 8, 1), axis=0))
            ev = kf_ref[pl.ds(0, TQ // 2, stride=2), :].reshape(TQ // 16, 1, 8, 128)
            od = kf_ref[pl.ds(1, TQ // 2, stride=2), :].reshape(TQ // 16, 1, 8, 128)
            kperm = jnp.concatenate([ev, od], axis=1).reshape(TQ, 128)
            for j in range(HPG):
                m = (lane >= j * DH) & (lane < (j + 1) * DH)
                kj = jnp.where(m, kperm, jnp.where(lane == BROW, 1.0, 0.0))
                kp_ref[j, pl.ds(pl.multiple_of(i * (TQ // 2), TQ // 2), TQ // 2), :] = _pack(
                    kj.astype(BF16))
            kv = kperm.reshape(TQ // CK, CK, 128)[:, :NV].reshape(NVB, 128)
            for d in range(DH):
                kb_ref[d, pl.ds(pl.multiple_of(i * NVB, NVB), NVB), :] = jnp.broadcast_to(
                    kv[:, d:d + 1], (NVB, 128))
            vt = jax.lax.dot_general(wvt_pad, xi, NT, preferred_element_type=F32)
            vt = vt.astype(BF16).astype(F32)
            vmax = jnp.maximum(vmax, jnp.abs(vt))
            vt_ref[0, :, rows] = jnp.where(vrow == DH, 1.0, vt)
            vtb = jnp.concatenate([vt[DH:], vt[:DH]], axis=0)
            vt_ref[1, :, rows] = jnp.where(vrow == 0, 1.0, vtb)
            qt = jax.lax.dot_general(_unpack(wqt_ref[...]), xi, NT,
                                     preferred_element_type=F32)
            for g in range(NG):
                n = min(HPG, H - g * HPG) * DH
                qg = qt[g * BROW: g * BROW + n]
                n2_ref[g, :, rows] = jnp.sum(qg * qg, axis=0, keepdims=True)
                blk = jnp.concatenate([qg, jnp.zeros((128 - n, TQ), F32)], axis=0).astype(BF16)
                qt_ref[i, g] = _pack(blk)
                qf_ref[i, g] = blk.astype(F32)
            return kmax2, vmax

        kmax2, vmax = jax.lax.fori_loop(
            0, NQB, chunk, (jnp.zeros((8, 1), F32), jnp.zeros((VROWS, TQ), F32)))
        for cp in late_copies:
            cp.start()
        k2 = jnp.max(kmax2) * (1.0 / HPG)
        shifts = [jnp.sqrt(n2_ref[g] * k2) * 1.02 for g in range(NG)]
        cmax = shifts[0]
        for c in shifts[1:]:
            cmax = jnp.maximum(cmax, c)
        safe = jnp.logical_and(jnp.max(cmax) <= SHIFT_MAX, jnp.max(vmax) >= VMIN)
        flag_ref[0] = safe.astype(jnp.int32)
        for g in range(NG):
            c = jnp.where(safe, shifts[g], 0.0)
            crow = pltpu.pack_elementwise([-c, jnp.zeros_like(c)], packed_dtype=BF16)
            cf = (-c).astype(BF16).astype(F32)
            for i in range(NQB):
                qt_ref[i, g, pl.ds(BROW // 2, 1), :] = crow[:, i * TQ:(i + 1) * TQ]
                qf_ref[i, g, pl.ds(BROW, 1), :] = cf[:, i * TQ:(i + 1) * TQ]
        build_qb(0)

    q0 = pl.multiple_of(step * TQ, TQ)
    safe = flag_ref[0] == 1

    def normalized(par, acc):
        row = 0 if par else DH
        return acc * (1.0 / acc[row:row + 1, :])

    def store_head(hp, par, o, cols):
        if par == 0:
            ot_ref[hp, pl.ds(0, VROWS), cols] = o
        else:
            row = jax.lax.broadcasted_iota(jnp.int32, (8, o.shape[1]), 0)
            ot_ref[hp, pl.ds(16, 8), cols] = jnp.where(row < 4, ot_ref[hp, pl.ds(16, 8), cols],
                                                       o[0:8])
            ot_ref[hp, pl.ds(VROWS, 2 * DH - VROWS), cols] = o[8:]

    @pl.when(safe)
    def _fast():
        def produce(g, j, c, slot):
            kc = _unpack(kp_ref[j, pl.ds((c * CK + NV) // 2, (CK - NV) // 2), :])
            q = _unpack(qt_ref[step, g])
            p_ref[slot] = _pk16(jnp.exp2(jnp.dot(kc, q, preferred_element_type=F32)))

        def vpu_rows(g, j, r0):
            acc = qb_ref[g, BROW]
            for d in range(DH):
                kb = kb_ref[d, pl.ds(r0, 8), :]
                acc = acc + jnp.concatenate([kb] * (TQ // 128), axis=1) * qb_ref[g, j * DH + d]
            return jnp.exp2(acc)

        def produce_v(g, j, c, slot):
            for b in range(NV // 16):
                e1 = vpu_rows(g, j, c * NV + b * 16)
                e2 = vpu_rows(g, j, c * NV + b * 16 + 8)
                pv_ref[slot, pl.ds(b * 8, 8), :] = pltpu.pack_elementwise([e1, e2],
                                                                          packed_dtype=BF16)

        def consume(j, c, t, acc):
            p = jnp.concatenate([pv_ref[t % NBV], p_ref[t % NBUF]], axis=0)
            return acc + jnp.dot(vt_ref[j % 2, :, pl.ds(c * CK, CK)], _unpack(p),
                                 preferred_element_type=F32)

        def group(g, nheads, g_next):
            t = 0
            for j in range(nheads):
                acc = jnp.zeros((VROWS, TQ), F32)
                for c in range(NCK):
                    for fn, la, nb in ((produce, LA, NBUF), (produce_v, LV, NBV)):
                        cn = c + la
                        slot = (t + la) % nb
                        if cn < NCK:
                            fn(g, j, cn, slot)
                        elif j + 1 < nheads:
                            fn(g, j + 1, cn - NCK, slot)
                        elif g_next is not None:
                            fn(g_next, 0, cn - NCK, slot)
                    acc = consume(j, c, t, acc)
                    t += 1
                store_head(g * (HPG // 2) + j // 2, j % 2, normalized(j % 2, acc),
                           slice(None))

        for c in range(LA):
            produce(0, 0, c, c % NBUF)
        for c in range(LV):
            produce_v(0, 0, c, c % NBV)

        def body(g, carry):
            group(g, HPG, g + 1)
            return carry

        jax.lax.fori_loop(0, NG - 1, body, 0)
        group(NG - 1, H - (NG - 1) * HPG, None)

    @pl.when(jnp.logical_not(safe))
    def _slow():
        def body(it, carry):
            hp = it // (TQ // 128)
            cols = pl.ds(pl.multiple_of((it % (TQ // 128)) * 128, 128), 128)
            g = hp // (HPG // 2)
            jp = hp % (HPG // 2)
            q = _unpack(qt_ref[step, g, :, cols])
            for par in range(2):
                s_ref[...] = jnp.dot(_unpack(kp_ref[2 * jp + par]), q,
                                     preferred_element_type=F32)
                m = jnp.max(s_ref[...], axis=0, keepdims=True)
                p = _unpack(_pk16(jnp.exp2(s_ref[...] - m)))
                acc = jnp.dot(vt_ref[par], p, preferred_element_type=F32)
                store_head(hp, par, normalized(par, acc), cols)
            return carry

        jax.lax.fori_loop(0, (H // 2) * (TQ // 128), body, 0)

    @pl.when(step == 0)
    def _wait_weights():
        for cp in late_copies:
            cp.wait()

    xb = x_ref[pl.ds(q0, TQ), :]
    b = jnp.zeros((TQ, D), F32)
    for f in range(FF // FC):
        gate = jnp.dot(xb, wg_ref[:, pl.ds(f * FC, FC)], preferred_element_type=F32)
        up = jnp.dot(xb, wu_ref[:, pl.ds(f * FC, FC)], preferred_element_type=F32)
        hh = (jnp.maximum(gate, 0.0) * up).astype(BF16)
        b = b + jnp.dot(hh, wd_ref[pl.ds(f * FC, FC), :], preferred_element_type=F32)

    build_qb(jnp.minimum(step + 1, NQB - 1))

    ot = ot_ref[...].reshape(D, TQ).astype(BF16)
    a = jax.lax.dot_general(ot, wo_ref[...], TN, preferred_element_type=F32)

    z = jnp.sum(xb.astype(F32) * gw_ref[:, pl.ds(0, D)].astype(F32), axis=-1, keepdims=True)
    g = 1.0 / (1.0 + jnp.exp(-z))
    o_ref[...] = (g * a + (1.0 - g) * b).astype(o_ref.dtype)


@jax.jit
def pallas_gated_mix__grouped_kv_mqa__glu_gated_reglu__prompt_kernel(
    A_x: jax.Array,
    A_wq: jax.Array,
    A_wk: jax.Array,
    A_wv: jax.Array,
    A_wo: jax.Array,
    B_x: jax.Array,
    B_W_gate: jax.Array,
    B_W_up: jax.Array,
    B_W_down: jax.Array,
    gate_w: jax.Array,
):
    x = A_x.reshape(S, D)
    gw = gate_w.reshape(1, D)

    out = pl.pallas_call(
        _kernel,
        grid=(NQB,),
        in_specs=[pl.BlockSpec(memory_space=pl.ANY)] * 9,
        out_specs=pl.BlockSpec((TQ, D), lambda i: (i, 0)),
        out_shape=jax.ShapeDtypeStruct((S, D), BF16),
        scratch_shapes=[
            pltpu.VMEM((S, D), BF16),
            pltpu.VMEM((D, D), BF16),
            pltpu.VMEM((D, D), BF16),
            pltpu.VMEM((D, FF), BF16),
            pltpu.VMEM((D, FF), BF16),
            pltpu.VMEM((FF, D), BF16),
            pltpu.VMEM((D // 2, D), U32),
            pltpu.VMEM((TQ, 128), F32),
            pltpu.VMEM((HPG, S // 2, 128), U32),
            pltpu.VMEM((DH, NCK * NV, 128), F32),
            pltpu.VMEM((2, VROWS, S), F32),
            pltpu.VMEM((NQB, NG, 64, TQ), U32),
            pltpu.VMEM((NQB, NG, 128, TQ), F32),
            pltpu.VMEM((NG, 128, 8, TQ), F32),
            pltpu.VMEM((NBUF, (CK - NV) // 2, TQ), U32),
            pltpu.VMEM((NBV, NV // 2, TQ), U32),
            pltpu.VMEM((S, 128), F32),
            pltpu.VMEM((H // 2, 2 * DH, TQ), F32),
            pltpu.VMEM((NG, 1, S), F32),
            pltpu.VMEM((DH, D), BF16),
            pltpu.VMEM((DH, D), BF16),
            pltpu.VMEM((1, 1024), BF16),
            pltpu.SMEM((1,), jnp.int32),
            pltpu.SemaphoreType.DMA((NQB + 8,)),
        ],
        compiler_params=pltpu.CompilerParams(
            dimension_semantics=("arbitrary",),
            vmem_limit_bytes=100 * 1024 * 1024,
        ),
    )(x, A_wq, A_wk.T, A_wv.T, gw, A_wo, B_W_gate, B_W_up, B_W_down)
    return out.reshape(1, S, D)
```

```python
import jax
import jax.numpy as jnp
import jax.experimental.pallas as pl
import jax.experimental.pallas.tpu as pltpu

F32 = jnp.float32
BF16 = jnp.bfloat16
U32 = jnp.uint32

S = 2048
D = 640
H = 32
DH = 20
FF = 1536
HPG = 6
NG = 6
BROW = HPG * DH
VROWS = 24
TQ = 512
NQB = S // TQ
CK = 128
NCK = S // CK
LA = 2
NBUF = LA + 1
FC = 512
NV_PAT = (16, 16, 16, 16)
NVS = [NV_PAT[c % len(NV_PAT)] for c in range(NCK)]
NMS = [CK - v for v in NVS]
VOFF = [sum(NVS[:c]) for c in range(NCK + 1)]
MOFF = [sum(NMS[:c]) for c in range(NCK + 1)]
NVB = sum(NV_PAT)
NMB = TQ - NVB
LV = 1
NBV = LV + 1
WROWS = D + 2 * VROWS
LOG2E = 1.4426950408889634
SHIFT_MAX = 48.0

NT = (((1,), (1,)), ((), ()))
TN = (((0,), (0,)), ((), ()))


def _pack(x_bf16):
    return pltpu.bitcast(x_bf16, U32)


def _unpack(x_u32):
    return pltpu.bitcast(x_u32, BF16)


def _pk16(e):
    n, w = e.shape
    e4 = e.reshape(n // 16, 2, 8, w)
    return pltpu.pack_elementwise([e4[:, 0], e4[:, 1]], packed_dtype=BF16).reshape(n // 2, w)


def _kernel(x_hbm, wq_hbm, wkt_hbm, wvt_hbm, gw_hbm, wo_hbm, wg_hbm, wu_hbm, wd_hbm,
            o_ref,
            x_ref, wq_ref, wo_ref, wg_ref, wu_ref, wd_ref,
            wt_ref, kf_ref, kpm_ref, kpv_ref, kb_ref, vt_ref, qt_ref, qf_ref, qb_ref, p_ref, pv_ref,
            s_ref, ot_ref, n2_ref, wkt_ref, wvt_ref, gw_ref, km_ref, flag_ref, sems):
    step = pl.program_id(0)

    def x_copy(i):
        rows = pl.ds(pl.multiple_of(i * TQ, TQ), TQ)
        return pltpu.make_async_copy(x_hbm.at[rows, :], x_ref.at[rows, :], sems.at[i])

    wk_copy = pltpu.make_async_copy(wkt_hbm, wkt_ref, sems.at[NQB])
    wv_copy = pltpu.make_async_copy(wvt_hbm, wvt_ref, sems.at[NQB + 1])
    wq_copy = pltpu.make_async_copy(wq_hbm, wq_ref, sems.at[NQB + 2])
    late_copies = (pltpu.make_async_copy(wo_hbm, wo_ref, sems.at[NQB + 3]),
                   pltpu.make_async_copy(wg_hbm, wg_ref, sems.at[NQB + 4]),
                   pltpu.make_async_copy(wu_hbm, wu_ref, sems.at[NQB + 5]),
                   pltpu.make_async_copy(wd_hbm, wd_ref, sems.at[NQB + 6]),
                   pltpu.make_async_copy(gw_hbm, gw_ref, sems.at[NQB + 7]))

    def build_qb_rows(qb, g, rows):
        for r in rows:
            qb_ref[g, r] = jnp.broadcast_to(qf_ref[qb, g, pl.ds(r, 1), :], (8, TQ))

    def build_qb(qb):
        for g in range(NG):
            n = min(HPG, H - g * HPG) * DH
            build_qb_rows(qb, g, list(range(n)) + [BROW])

    @pl.when(step == 0)
    def _setup():
        wq_copy.start()
        wk_copy.start()
        wv_copy.start()
        for i in range(NQB):
            x_copy(i).start()

        wq_copy.wait()
        wt_ref[pl.ds(0, D // 2), :] = _pack(wq_ref[...].astype(F32).T.astype(BF16))
        wk_copy.wait()
        wv_copy.wait()
        zpad = jnp.zeros((VROWS - DH, D), F32)
        wkv = jnp.concatenate([wkt_ref[...].astype(F32), zpad,
                               wvt_ref[...].astype(F32), zpad], axis=0)
        wt_ref[pl.ds(D // 2, VROWS), :] = _pack(wkv.astype(BF16))

        def chunk(i, vmax, qb_groups):
            x_copy(i).wait()
            for g in qb_groups:
                build_qb_rows(0, g, range(BROW))
            rows = pl.ds(pl.multiple_of(i * TQ, TQ), TQ)
            lane = jax.lax.broadcasted_iota(jnp.int32, (TQ, 128), 1)
            vrow = jax.lax.broadcasted_iota(jnp.int32, (VROWS, TQ), 0)
            xi = x_ref[rows, :]
            kvt = jax.lax.dot_general(_unpack(wt_ref[pl.ds(D // 2, VROWS), :]), xi, NT,
                                      preferred_element_type=F32)
            kt = (kvt[:VROWS] * (DH ** -0.5 * LOG2E)).astype(BF16).astype(F32)
            km_ref[...] = jnp.maximum(km_ref[...], jnp.sum(kt * kt, axis=0, keepdims=True))
            krept = jnp.concatenate([kt[:DH]] * HPG + [jnp.zeros((128 - BROW, TQ), F32)], axis=0)
            kf_ref[...] = krept.T
            ev = kf_ref[pl.ds(0, TQ // 2, stride=2), :].reshape(TQ // 16, 1, 8, 128)
            od = kf_ref[pl.ds(1, TQ // 2, stride=2), :].reshape(TQ // 16, 1, 8, 128)
            kperm = jnp.concatenate([ev, od], axis=1).reshape(TQ, 128)
            for j in range(HPG):
                m = (lane >= j * DH) & (lane < (j + 1) * DH)
                kj = jnp.where(m, kperm, jnp.where(lane == BROW, 1.0, 0.0))
                kj = _pack(kj.astype(BF16))
                kpv_ref[j, pl.ds(pl.multiple_of(i * (NVB // 2), 8), NVB // 2), :] = (
                    jnp.concatenate([kj[c * CK // 2:(c * CK + NV_PAT[c]) // 2]
                                     for c in range(TQ // CK)], axis=0))
                kpm_ref[j, pl.ds(pl.multiple_of(i * (NMB // 2), 8), NMB // 2), :] = (
                    jnp.concatenate([kj[(c * CK + NV_PAT[c]) // 2:(c + 1) * CK // 2]
                                     for c in range(TQ // CK)], axis=0))
            kv = jnp.concatenate([kperm[c * CK:c * CK + NV_PAT[c]] for c in range(TQ // CK)],
                                 axis=0)
            for d in range(DH):
                kb_ref[d, pl.ds(pl.multiple_of(i * NVB, 16), NVB), :] = jnp.broadcast_to(
                    kv[:, d:d + 1], (NVB, 128))
            vt = kvt[VROWS:].astype(BF16).astype(F32)
            vmax = jnp.maximum(vmax, jnp.abs(vt))
            vt_ref[0, :, rows] = jnp.where(vrow == DH, 1.0, vt)
            vtb = jnp.concatenate([vt[DH:], vt[:DH]], axis=0)
            vt_ref[1, :, rows] = jnp.where(vrow == 0, 1.0, vtb)
            proj = jax.lax.dot_general(_unpack(wt_ref[pl.ds(0, D // 2), :]), xi, NT,
                                       preferred_element_type=F32)
            for g in range(NG):
                n = min(HPG, H - g * HPG) * DH
                qg = proj[g * BROW: g * BROW + n]
                n2_ref[g, :, rows] = jnp.sum(qg * qg, axis=0, keepdims=True)
                blk = jnp.concatenate([qg, jnp.zeros((128 - n, TQ), F32)], axis=0).astype(BF16)
                qt_ref[i, g] = _pack(blk)
                qf_ref[i, g] = blk.astype(F32)
            return vmax

        km_ref[...] = jnp.zeros((1, TQ), F32)
        carry = chunk(0, jnp.zeros((VROWS, TQ), F32), ())
        gpi = NG // (NQB - 1)
        vmax = jax.lax.fori_loop(
            1, NQB,
            lambda i, c: chunk(i, c, [(i - 1) * gpi + u for u in range(gpi)]), carry)
        for cp in late_copies:
            cp.start()
        k2 = jnp.max(km_ref[...])
        shifts = [jnp.sqrt(n2_ref[g] * k2) * 1.02 for g in range(NG)]
        cmax = shifts[0]
        for c in shifts[1:]:
            cmax = jnp.maximum(cmax, c)
        cm = jnp.max(cmax, axis=1, keepdims=True)
        vm = jnp.max(jnp.max(vmax, axis=0, keepdims=True), axis=1, keepdims=True)
        ok = jnp.logical_and(cm <= SHIFT_MAX, vm >= jnp.exp2(2.0 * cm - 100.0))
        safe = jnp.max(ok.astype(jnp.int32)) == 1
        flag_ref[0] = safe.astype(jnp.int32)
        for g in range(NG):
            c = jnp.where(safe, shifts[g], 0.0)
            crow = pltpu.pack_elementwise([-c, jnp.zeros_like(c)], packed_dtype=BF16)
            cf = (-c).astype(BF16).astype(F32)
            for i in range(NQB):
                qt_ref[i, g, pl.ds(BROW // 2, 1), :] = crow[:, i * TQ:(i + 1) * TQ]
                qf_ref[i, g, pl.ds(BROW, 1), :] = cf[:, i * TQ:(i + 1) * TQ]
            build_qb_rows(0, g, [BROW])

    q0 = pl.multiple_of(step * TQ, TQ)
    safe = flag_ref[0] == 1

    def normalized(par, acc):
        row = 0 if par else DH
        return acc * (1.0 / acc[row:row + 1, :])

    def store_head(hp, par, o, cols):
        if par == 0:
            ot_ref[hp, pl.ds(0, VROWS), cols] = o
        else:
            row = jax.lax.broadcasted_iota(jnp.int32, (8, o.shape[1]), 0)
            ot_ref[hp, pl.ds(16, 8), cols] = jnp.where(row < 4, ot_ref[hp, pl.ds(16, 8), cols],
                                                       o[0:8])
            ot_ref[hp, pl.ds(VROWS, 2 * DH - VROWS), cols] = o[8:]

    @pl.when(safe)
    def _fast():
        def produce(g, j, c, t):
            kc = _unpack(kpm_ref[j, pl.ds(MOFF[c] // 2, NMS[c] // 2), :])
            q = _unpack(qt_ref[step, g])
            p_ref[t % NBUF, pl.ds(0, NMS[c] // 2), :] = _pk16(
                jnp.exp2(jnp.dot(kc, q, preferred_element_type=F32)))

        def vpu_rows(g, j, r0):
            acc = qb_ref[g, BROW]
            for d in range(DH):
                kb = kb_ref[d, pl.ds(r0, 8), :]
                acc = acc + jnp.concatenate([kb] * (TQ // 128), axis=1) * qb_ref[g, j * DH + d]
            return jnp.exp2(acc)

        def produce_v(g, j, c, t):
            slot = t % NBV
            for b in range(NVS[c] // 16):
                e2 = vpu_rows(g, j, VOFF[c] + b * 16 + 8)
                e1 = vpu_rows(g, j, VOFF[c] + b * 16)
                pv_ref[slot, pl.ds(b * 8, 8), :] = pltpu.pack_elementwise([e1, e2],
                                                                          packed_dtype=BF16)

        def consume(j, c, t, acc):
            p = jnp.concatenate([pv_ref[t % NBV, pl.ds(0, NVS[c] // 2), :],
                                 p_ref[t % NBUF, pl.ds(0, NMS[c] // 2), :]], axis=0)
            return acc + jnp.dot(vt_ref[j % 2, :, pl.ds(c * CK, CK)], _unpack(p),
                                 preferred_element_type=F32)

        def group(g, nheads, g_next):
            t = 0
            for j in range(nheads):
                acc = jnp.zeros((VROWS, TQ), F32)
                for c in range(NCK):
                    for fn, la in ((produce, LA), (produce_v, LV)):
                        cn = c + la
                        if cn < NCK:
                            fn(g, j, cn, t + la)
                        elif j + 1 < nheads:
                            fn(g, j + 1, cn - NCK, t + la)
                        elif g_next is not None:
                            fn(g_next, 0, cn - NCK, t + la)
                    acc = consume(j, c, t, acc)
                    t += 1
                store_head(g * (HPG // 2) + j // 2, j % 2, normalized(j % 2, acc),
                           slice(None))

        for c in range(LA):
            produce(0, 0, c, c)
        for c in range(LV):
            produce_v(0, 0, c, c)

        def body(g, carry):
            group(g, HPG, g + 1)
            return carry

        jax.lax.fori_loop(0, NG - 1, body, 0)
        group(NG - 1, H - (NG - 1) * HPG, None)

    @pl.when(jnp.logical_not(safe))
    def _slow():
        def body(it, carry):
            hp = it // (TQ // 128)
            cols = pl.ds(pl.multiple_of((it % (TQ // 128)) * 128, 128), 128)
            g = hp // (HPG // 2)
            jp = hp % (HPG // 2)
            q = _unpack(qt_ref[step, g, :, cols])
            nvk = VOFF[NCK]
            for par in range(2):
                j = 2 * jp + par
                s_ref[pl.ds(0, nvk), :] = jnp.dot(_unpack(kpv_ref[j]), q,
                                                  preferred_element_type=F32)
                s_ref[pl.ds(nvk, S - nvk), :] = jnp.dot(_unpack(kpm_ref[j]), q,
                                                        preferred_element_type=F32)
                m = jnp.max(s_ref[...], axis=0, keepdims=True)
                e = _pk16(jnp.exp2(s_ref[...] - m))
                pieces = []
                for c in range(NCK):
                    pieces += [e[VOFF[c] // 2:VOFF[c + 1] // 2],
                               e[(nvk + MOFF[c]) // 2:(nvk + MOFF[c + 1]) // 2]]
                p = _unpack(jnp.concatenate(pieces, axis=0))
                acc = jnp.dot(vt_ref[par], p, preferred_element_type=F32)
                store_head(hp, par, normalized(par, acc), cols)
            return carry

        jax.lax.fori_loop(0, (H // 2) * (TQ // 128), body, 0)

    @pl.when(step == 0)
    def _wait_weights():
        for cp in late_copies:
            cp.wait()

    xb = x_ref[pl.ds(q0, TQ), :]
    b = jnp.zeros((TQ, D), F32)
    for f in range(FF // FC):
        gate = jnp.dot(xb, wg_ref[:, pl.ds(f * FC, FC)], preferred_element_type=F32)
        up = jnp.dot(xb, wu_ref[:, pl.ds(f * FC, FC)], preferred_element_type=F32)
        hh = (jnp.maximum(gate, 0.0) * up).astype(BF16)
        b = b + jnp.dot(hh, wd_ref[pl.ds(f * FC, FC), :], preferred_element_type=F32)

    build_qb(jnp.minimum(step + 1, NQB - 1))

    ot = ot_ref[...].reshape(D, TQ).astype(BF16)
    a = jax.lax.dot_general(ot, wo_ref[...], TN, preferred_element_type=F32)

    gw = gw_ref[...].astype(F32)
    xf = xb.astype(F32)
    zp = xf[:, 0:128] * gw[0:1]
    for t in range(1, D // 128):
        zp = zp + xf[:, t * 128:(t + 1) * 128] * gw[t:t + 1]
    z = jnp.sum(zp, axis=-1, keepdims=True)
    g = 1.0 / (1.0 + jnp.exp(-z))
    o_ref[...] = (g * a + (1.0 - g) * b).astype(o_ref.dtype)


@jax.jit
def pallas_gated_mix__grouped_kv_mqa__glu_gated_reglu__prompt_kernel(
    A_x: jax.Array,
    A_wq: jax.Array,
    A_wk: jax.Array,
    A_wv: jax.Array,
    A_wo: jax.Array,
    B_x: jax.Array,
    B_W_gate: jax.Array,
    B_W_up: jax.Array,
    B_W_down: jax.Array,
    gate_w: jax.Array,
):
    x = A_x.reshape(S, D)
    gw = gate_w.reshape(D // 128, 128)

    out = pl.pallas_call(
        _kernel,
        grid=(NQB,),
        in_specs=[pl.BlockSpec(memory_space=pl.ANY)] * 9,
        out_specs=pl.BlockSpec((TQ, D), lambda i: (i, 0)),
        out_shape=jax.ShapeDtypeStruct((S, D), BF16),
        scratch_shapes=[
            pltpu.VMEM((S, D), BF16),
            pltpu.VMEM((D, D), BF16),
            pltpu.VMEM((D, D), BF16),
            pltpu.VMEM((D, FF), BF16),
            pltpu.VMEM((D, FF), BF16),
            pltpu.VMEM((FF, D), BF16),
            pltpu.VMEM((WROWS // 2 + 8, D), U32),
            pltpu.VMEM((TQ, 128), F32),
            pltpu.VMEM((HPG, MOFF[NCK] // 2, 128), U32),
            pltpu.VMEM((HPG, VOFF[NCK] // 2, 128), U32),
            pltpu.VMEM((DH, VOFF[NCK], 128), F32),
            pltpu.VMEM((2, VROWS, S), F32),
            pltpu.VMEM((NQB, NG, 64, TQ), U32),
            pltpu.VMEM((NQB, NG, 128, TQ), F32),
            pltpu.VMEM((NG, 128, 8, TQ), F32),
            pltpu.VMEM((NBUF, CK // 2, TQ), U32),
            pltpu.VMEM((NBV, 16, TQ), U32),
            pltpu.VMEM((S, 128), F32),
            pltpu.VMEM((H // 2, 2 * DH, TQ), F32),
            pltpu.VMEM((NG, 1, S), F32),
            pltpu.VMEM((DH, D), BF16),
            pltpu.VMEM((DH, D), BF16),
            pltpu.VMEM((D // 128, 128), BF16),
            pltpu.VMEM((1, TQ), F32),
            pltpu.SMEM((1,), jnp.int32),
            pltpu.SemaphoreType.DMA((NQB + 8,)),
        ],
        compiler_params=pltpu.CompilerParams(
            dimension_semantics=("arbitrary",),
            vmem_limit_bytes=100 * 1024 * 1024,
        ),
    )(x, A_wq, A_wk.T, A_wv.T, gw, A_wo, B_W_gate, B_W_up, B_W_down)
    return out.reshape(1, S, D)
```

```python
import jax
import jax.numpy as jnp
import jax.experimental.pallas as pl
import jax.experimental.pallas.tpu as pltpu

F32 = jnp.float32
BF16 = jnp.bfloat16
U32 = jnp.uint32

S = 2048
D = 640
H = 32
DH = 20
FF = 1536
HPG = 6
NG = 6
BROW = HPG * DH
VROWS = 24
TQ = 512
NQB = S // TQ
CK = 128
NCK = S // CK
LA = 2
NBUF = LA + 1
FC = 512
NV_PAT = (16, 16, 16, 16)
NVS = [NV_PAT[c % len(NV_PAT)] for c in range(NCK)]
NMS = [CK - v for v in NVS]
VOFF = [sum(NVS[:c]) for c in range(NCK + 1)]
MOFF = [sum(NMS[:c]) for c in range(NCK + 1)]
NVB = sum(NV_PAT)
NMB = TQ - NVB
LV = 1
NBV = LV + 1
WROWS = D + 2 * VROWS
LOG2E = 1.4426950408889634
SHIFT_MAX = 48.0

NT = (((1,), (1,)), ((), ()))
TN = (((0,), (0,)), ((), ()))


def _pack(x_bf16):
    return pltpu.bitcast(x_bf16, U32)


def _unpack(x_u32):
    return pltpu.bitcast(x_u32, BF16)


def _pk16(e):
    n, w = e.shape
    e4 = e.reshape(n // 16, 2, 8, w)
    return pltpu.pack_elementwise([e4[:, 0], e4[:, 1]], packed_dtype=BF16).reshape(n // 2, w)


def _kernel(x_hbm, wq_hbm, wkt_hbm, wvt_hbm, gw_hbm, wo_hbm, wg_hbm, wu_hbm, wd_hbm,
            o_ref,
            x_ref, wq_ref, wo_ref, wg_ref, wu_ref, wd_ref,
            wt_ref, kf_ref, kpm_ref, kpv_ref, kb_ref, vt_ref, qt_ref, qf_ref, qb_ref, p_ref, pv_ref,
            s_ref, ot_ref, acc_ref, n2_ref, wkt_ref, wvt_ref, gw_ref, km_ref, flag_ref, sems):
    step = pl.program_id(0)

    def x_copy(i):
        rows = pl.ds(pl.multiple_of(i * TQ, TQ), TQ)
        return pltpu.make_async_copy(x_hbm.at[rows, :], x_ref.at[rows, :], sems.at[i])

    wk_copy = pltpu.make_async_copy(wkt_hbm, wkt_ref, sems.at[NQB])
    wv_copy = pltpu.make_async_copy(wvt_hbm, wvt_ref, sems.at[NQB + 1])
    wq_copy = pltpu.make_async_copy(wq_hbm, wq_ref, sems.at[NQB + 2])
    late_copies = (pltpu.make_async_copy(wo_hbm, wo_ref, sems.at[NQB + 3]),
                   pltpu.make_async_copy(wg_hbm, wg_ref, sems.at[NQB + 4]),
                   pltpu.make_async_copy(wu_hbm, wu_ref, sems.at[NQB + 5]),
                   pltpu.make_async_copy(wd_hbm, wd_ref, sems.at[NQB + 6]),
                   pltpu.make_async_copy(gw_hbm, gw_ref, sems.at[NQB + 7]))

    def build_qb_rows(qb, g, rows):
        for r in rows:
            qb_ref[g, r] = jnp.broadcast_to(qf_ref[qb, g, pl.ds(r, 1), :], (8, TQ))

    def build_qb(qb):
        for g in range(NG):
            n = min(HPG, H - g * HPG) * DH
            build_qb_rows(qb, g, list(range(n)) + [BROW])

    @pl.when(step == 0)
    def _setup():
        wq_copy.start()
        wk_copy.start()
        wv_copy.start()
        for i in range(NQB):
            x_copy(i).start()

        wq_copy.wait()
        wt_ref[pl.ds(0, D // 2), :] = _pack(wq_ref[...].astype(F32).T.astype(BF16))
        wk_copy.wait()
        wv_copy.wait()
        zpad = jnp.zeros((VROWS - DH, D), F32)
        wkv = jnp.concatenate([wkt_ref[...].astype(F32), zpad,
                               wvt_ref[...].astype(F32), zpad], axis=0)
        wt_ref[pl.ds(D // 2, VROWS), :] = _pack(wkv.astype(BF16))

        def chunk(i, vmax, qb_groups):
            x_copy(i).wait()
            for g in qb_groups:
                build_qb_rows(0, g, range(BROW))
            rows = pl.ds(pl.multiple_of(i * TQ, TQ), TQ)
            lane = jax.lax.broadcasted_iota(jnp.int32, (TQ, 128), 1)
            vrow = jax.lax.broadcasted_iota(jnp.int32, (VROWS, TQ), 0)
            xi = x_ref[rows, :]
            kvt = jax.lax.dot_general(_unpack(wt_ref[pl.ds(D // 2, VROWS), :]), xi, NT,
                                      preferred_element_type=F32)
            kt = (kvt[:VROWS] * (DH ** -0.5 * LOG2E)).astype(BF16).astype(F32)
            km_ref[...] = jnp.maximum(km_ref[...], jnp.sum(kt * kt, axis=0, keepdims=True))
            krept = jnp.concatenate([kt[:DH]] * HPG + [jnp.zeros((128 - BROW, TQ), F32)], axis=0)
            kf_ref[...] = krept.T
            ev = kf_ref[pl.ds(0, TQ // 2, stride=2), :].reshape(TQ // 16, 1, 8, 128)
            od = kf_ref[pl.ds(1, TQ // 2, stride=2), :].reshape(TQ // 16, 1, 8, 128)
            kperm = jnp.concatenate([ev, od], axis=1).reshape(TQ, 128)
            for j in range(HPG):
                m = (lane >= j * DH) & (lane < (j + 1) * DH)
                kj = jnp.where(m, kperm, jnp.where(lane == BROW, 1.0, 0.0))
                kj = _pack(kj.astype(BF16))
                kpv_ref[j, pl.ds(pl.multiple_of(i * (NVB // 2), 8), NVB // 2), :] = (
                    jnp.concatenate([kj[c * CK // 2:(c * CK + NV_PAT[c]) // 2]
                                     for c in range(TQ // CK)], axis=0))
                kpm_ref[j, pl.ds(pl.multiple_of(i * (NMB // 2), 8), NMB // 2), :] = (
                    jnp.concatenate([kj[(c * CK + NV_PAT[c]) // 2:(c + 1) * CK // 2]
                                     for c in range(TQ // CK)], axis=0))
            kv = jnp.concatenate([kperm[c * CK:c * CK + NV_PAT[c]] for c in range(TQ // CK)],
                                 axis=0)
            for d in range(DH):
                kb_ref[d, pl.ds(pl.multiple_of(i * NVB, 16), NVB), :] = jnp.broadcast_to(
                    kv[:, d:d + 1], (NVB, 128))
            vt = kvt[VROWS:].astype(BF16).astype(F32)
            vmax = jnp.maximum(vmax, jnp.abs(vt))
            vt_ref[0, :, rows] = jnp.where(vrow == DH, 1.0, vt)
            vtb = jnp.concatenate([vt[DH:], vt[:DH]], axis=0)
            vt_ref[1, :, rows] = jnp.where(vrow == 0, 1.0, vtb)
            proj = jax.lax.dot_general(_unpack(wt_ref[pl.ds(0, D // 2), :]), xi, NT,
                                       preferred_element_type=F32)
            for g in range(NG):
                n = min(HPG, H - g * HPG) * DH
                qg = proj[g * BROW: g * BROW + n]
                n2_ref[g, :, rows] = jnp.sum(qg * qg, axis=0, keepdims=True)
                blk = jnp.concatenate([qg, jnp.zeros((128 - n, TQ), F32)], axis=0).astype(BF16)
                qt_ref[i, g] = _pack(blk)
                qf_ref[i, g] = blk.astype(F32)
            return vmax

        km_ref[...] = jnp.zeros((1, TQ), F32)
        carry = chunk(0, jnp.zeros((VROWS, TQ), F32), ())
        gpi = NG // (NQB - 1)
        vmax = jax.lax.fori_loop(
            1, NQB,
            lambda i, c: chunk(i, c, [(i - 1) * gpi + u for u in range(gpi)]), carry)
        for cp in late_copies:
            cp.start()
        k2 = jnp.max(km_ref[...])
        shifts = [jnp.sqrt(n2_ref[g] * k2) * 1.02 for g in range(NG)]
        cmax = shifts[0]
        for c in shifts[1:]:
            cmax = jnp.maximum(cmax, c)
        cm = jnp.max(cmax, axis=1, keepdims=True)
        vm = jnp.max(jnp.max(vmax, axis=0, keepdims=True), axis=1, keepdims=True)
        ok = jnp.logical_and(cm <= SHIFT_MAX, vm >= jnp.exp2(2.0 * cm - 100.0))
        safe = jnp.max(ok.astype(jnp.int32)) == 1
        flag_ref[0] = safe.astype(jnp.int32)
        for g in range(NG):
            c = jnp.where(safe, shifts[g], 0.0)
            crow = pltpu.pack_elementwise([-c, jnp.zeros_like(c)], packed_dtype=BF16)
            cf = (-c).astype(BF16).astype(F32)
            for i in range(NQB):
                qt_ref[i, g, pl.ds(BROW // 2, 1), :] = crow[:, i * TQ:(i + 1) * TQ]
                qf_ref[i, g, pl.ds(BROW, 1), :] = cf[:, i * TQ:(i + 1) * TQ]
            build_qb_rows(0, g, [BROW])

    q0 = pl.multiple_of(step * TQ, TQ)
    safe = flag_ref[0] == 1

    def normalized(par, acc):
        row = 0 if par else DH
        return acc * (1.0 / acc[row:row + 1, :])

    def store_head(hp, par, o, cols):
        if par == 0:
            ot_ref[hp, pl.ds(0, VROWS), cols] = o
        else:
            row = jax.lax.broadcasted_iota(jnp.int32, (8, o.shape[1]), 0)
            ot_ref[hp, pl.ds(16, 8), cols] = jnp.where(row < 4, ot_ref[hp, pl.ds(16, 8), cols],
                                                       o[0:8])
            ot_ref[hp, pl.ds(VROWS, 2 * DH - VROWS), cols] = o[8:]

    @pl.when(safe)
    def _fast():
        def produce(g, j, c, t):
            kc = _unpack(kpm_ref[j, pl.ds(MOFF[c] // 2, NMS[c] // 2), :])
            q = _unpack(qt_ref[step, g])
            p_ref[t % NBUF, pl.ds(0, NMS[c] // 2), :] = _pk16(
                jnp.exp2(jnp.dot(kc, q, preferred_element_type=F32)))

        def vpu_rows(g, j, r0):
            acc = qb_ref[g, BROW]
            for d in range(DH):
                kb = kb_ref[d, pl.ds(r0, 8), :]
                acc = acc + jnp.concatenate([kb] * (TQ // 128), axis=1) * qb_ref[g, j * DH + d]
            return jnp.exp2(acc)

        def produce_v(g, j, c, t):
            slot = t % NBV
            for b in range(NVS[c] // 16):
                e2 = vpu_rows(g, j, VOFF[c] + b * 16 + 8)
                e1 = vpu_rows(g, j, VOFF[c] + b * 16)
                pv_ref[slot, pl.ds(b * 8, 8), :] = pltpu.pack_elementwise([e1, e2],
                                                                          packed_dtype=BF16)

        def consume(j, c, t, acc):
            p = jnp.concatenate([pv_ref[t % NBV, pl.ds(0, NVS[c] // 2), :],
                                 p_ref[t % NBUF, pl.ds(0, NMS[c] // 2), :]], axis=0)
            return acc + jnp.dot(vt_ref[j % 2, :, pl.ds(c * CK, CK)], _unpack(p),
                                 preferred_element_type=F32)

        def group(g, nheads, g_next):
            items = [(c, j) for c in range(NCK) for j in range(nheads)]
            n = len(items)
            for t, (c, j) in enumerate(items):
                for fn, la in ((produce, LA), (produce_v, LV)):
                    tn = t + la
                    if tn < n:
                        cn, jn = items[tn]
                        fn(g, jn, cn, tn)
                    elif g_next is not None:
                        fn(g_next, tn - n, 0, tn)
                p = jnp.concatenate([pv_ref[t % NBV, pl.ds(0, NVS[c] // 2), :],
                                     p_ref[t % NBUF, pl.ds(0, NMS[c] // 2), :]], axis=0)
                r = jnp.dot(vt_ref[j % 2, :, pl.ds(c * CK, CK)], _unpack(p),
                            preferred_element_type=F32)
                if c == 0:
                    acc_ref[j, pl.ds(0, VROWS), :] = r
                elif c < NCK - 1:
                    acc_ref[j, pl.ds(0, VROWS), :] = acc_ref[j, pl.ds(0, VROWS), :] + r
                else:
                    acc = acc_ref[j, pl.ds(0, VROWS), :] + r
                    store_head(g * (HPG // 2) + j // 2, j % 2, normalized(j % 2, acc),
                               slice(None))

        for c in range(LA):
            produce(0, c, 0, c)
        for c in range(LV):
            produce_v(0, c, 0, c)

        def body(g, carry):
            group(g, HPG, g + 1)
            return carry

        jax.lax.fori_loop(0, NG - 1, body, 0)
        group(NG - 1, H - (NG - 1) * HPG, None)

    @pl.when(jnp.logical_not(safe))
    def _slow():
        def body(it, carry):
            hp = it // (TQ // 128)
            cols = pl.ds(pl.multiple_of((it % (TQ // 128)) * 128, 128), 128)
            g = hp // (HPG // 2)
            jp = hp % (HPG // 2)
            q = _unpack(qt_ref[step, g, :, cols])
            nvk = VOFF[NCK]
            for par in range(2):
                j = 2 * jp + par
                s_ref[pl.ds(0, nvk), :] = jnp.dot(_unpack(kpv_ref[j]), q,
                                                  preferred_element_type=F32)
                s_ref[pl.ds(nvk, S - nvk), :] = jnp.dot(_unpack(kpm_ref[j]), q,
                                                        preferred_element_type=F32)
                m = jnp.max(s_ref[...], axis=0, keepdims=True)
                e = _pk16(jnp.exp2(s_ref[...] - m))
                pieces = []
                for c in range(NCK):
                    pieces += [e[VOFF[c] // 2:VOFF[c + 1] // 2],
                               e[(nvk + MOFF[c]) // 2:(nvk + MOFF[c + 1]) // 2]]
                p = _unpack(jnp.concatenate(pieces, axis=0))
                acc = jnp.dot(vt_ref[par], p, preferred_element_type=F32)
                store_head(hp, par, normalized(par, acc), cols)
            return carry

        jax.lax.fori_loop(0, (H // 2) * (TQ // 128), body, 0)

    @pl.when(step == 0)
    def _wait_weights():
        for cp in late_copies:
            cp.wait()

    xb = x_ref[pl.ds(q0, TQ), :]
    b = jnp.zeros((TQ, D), F32)
    for f in range(FF // FC):
        gate = jnp.dot(xb, wg_ref[:, pl.ds(f * FC, FC)], preferred_element_type=F32)
        up = jnp.dot(xb, wu_ref[:, pl.ds(f * FC, FC)], preferred_element_type=F32)
        hh = (jnp.maximum(gate, 0.0) * up).astype(BF16)
        b = b + jnp.dot(hh, wd_ref[pl.ds(f * FC, FC), :], preferred_element_type=F32)

    build_qb(jnp.minimum(step + 1, NQB - 1))

    ot = ot_ref[...].reshape(D, TQ).astype(BF16)
    a = jax.lax.dot_general(ot, wo_ref[...], TN, preferred_element_type=F32)

    gw = gw_ref[...].astype(F32)
    xf = xb.astype(F32)
    zp = xf[:, 0:128] * gw[0:1]
    for t in range(1, D // 128):
        zp = zp + xf[:, t * 128:(t + 1) * 128] * gw[t:t + 1]
    z = jnp.sum(zp, axis=-1, keepdims=True)
    g = 1.0 / (1.0 + jnp.exp(-z))
    o_ref[...] = (g * a + (1.0 - g) * b).astype(o_ref.dtype)


@jax.jit
def pallas_gated_mix__grouped_kv_mqa__glu_gated_reglu__prompt_kernel(
    A_x: jax.Array,
    A_wq: jax.Array,
    A_wk: jax.Array,
    A_wv: jax.Array,
    A_wo: jax.Array,
    B_x: jax.Array,
    B_W_gate: jax.Array,
    B_W_up: jax.Array,
    B_W_down: jax.Array,
    gate_w: jax.Array,
):
    x = A_x.reshape(S, D)
    gw = gate_w.reshape(D // 128, 128)

    out = pl.pallas_call(
        _kernel,
        grid=(NQB,),
        in_specs=[pl.BlockSpec(memory_space=pl.ANY)] * 9,
        out_specs=pl.BlockSpec((TQ, D), lambda i: (i, 0)),
        out_shape=jax.ShapeDtypeStruct((S, D), BF16),
        scratch_shapes=[
            pltpu.VMEM((S, D), BF16),
            pltpu.VMEM((D, D), BF16),
            pltpu.VMEM((D, D), BF16),
            pltpu.VMEM((D, FF), BF16),
            pltpu.VMEM((D, FF), BF16),
            pltpu.VMEM((FF, D), BF16),
            pltpu.VMEM((WROWS // 2 + 8, D), U32),
            pltpu.VMEM((TQ, 128), F32),
            pltpu.VMEM((HPG, MOFF[NCK] // 2, 128), U32),
            pltpu.VMEM((HPG, VOFF[NCK] // 2, 128), U32),
            pltpu.VMEM((DH, VOFF[NCK], 128), F32),
            pltpu.VMEM((2, VROWS, S), F32),
            pltpu.VMEM((NQB, NG, 64, TQ), U32),
            pltpu.VMEM((NQB, NG, 128, TQ), F32),
            pltpu.VMEM((NG, 128, 8, TQ), F32),
            pltpu.VMEM((NBUF, CK // 2, TQ), U32),
            pltpu.VMEM((NBV, 16, TQ), U32),
            pltpu.VMEM((S, 128), F32),
            pltpu.VMEM((H // 2, 2 * DH, TQ), F32),
            pltpu.VMEM((HPG, VROWS + 8, TQ), F32),
            pltpu.VMEM((NG, 1, S), F32),
            pltpu.VMEM((DH, D), BF16),
            pltpu.VMEM((DH, D), BF16),
            pltpu.VMEM((D // 128, 128), BF16),
            pltpu.VMEM((1, TQ), F32),
            pltpu.SMEM((1,), jnp.int32),
            pltpu.SemaphoreType.DMA((NQB + 8,)),
        ],
        compiler_params=pltpu.CompilerParams(
            dimension_semantics=("arbitrary",),
            vmem_limit_bytes=100 * 1024 * 1024,
        ),
    )(x, A_wq, A_wk.T, A_wv.T, gw, A_wo, B_W_gate, B_W_up, B_W_down)
    return out.reshape(1, S, D)
```

```python
import jax
import jax.numpy as jnp
import jax.experimental.pallas as pl
import jax.experimental.pallas.tpu as pltpu

F32 = jnp.float32
BF16 = jnp.bfloat16
U32 = jnp.uint32

S = 2048
D = 640
H = 32
DH = 20
FF = 1536
HPG = 6
NG = 6
BROW = HPG * DH
VROWS = 24
TQ = 512
NQB = S // TQ
CK = 128
NCK = S // CK
LA = 2
NBUF = LA + 1
FC = 512
NV_PAT = (16, 16, 16, 16)
NVS = [NV_PAT[c % len(NV_PAT)] for c in range(NCK)]
NMS = [CK - v for v in NVS]
VOFF = [sum(NVS[:c]) for c in range(NCK + 1)]
MOFF = [sum(NMS[:c]) for c in range(NCK + 1)]
NVB = sum(NV_PAT)
NMB = TQ - NVB
LV = 1
NBV = LV + 1
WROWS = D + 2 * VROWS
LOG2E = 1.4426950408889634
SHIFT_MAX = 48.0

NT = (((1,), (1,)), ((), ()))
TN = (((0,), (0,)), ((), ()))


def _pack(x_bf16):
    return pltpu.bitcast(x_bf16, U32)


def _unpack(x_u32):
    return pltpu.bitcast(x_u32, BF16)


def _pk16(e):
    n, w = e.shape
    e4 = e.reshape(n // 16, 2, 8, w)
    return pltpu.pack_elementwise([e4[:, 0], e4[:, 1]], packed_dtype=BF16).reshape(n // 2, w)


def _kernel(x_hbm, wq_hbm, wkt_hbm, wvt_hbm, gw_hbm, wo_hbm, wg_hbm, wu_hbm, wd_hbm,
            o_ref,
            x_ref, wq_ref, wo_ref, wg_ref, wu_ref, wd_ref,
            wt_ref, kf_ref, kpm_ref, kpv_ref, kb_ref, vt_ref, qt_ref, qf_ref, qb_ref, p_ref, pv_ref,
            s_ref, ot_ref, acc_ref, n2_ref, wkt_ref, wvt_ref, gw_ref, km_ref, flag_ref, sems):
    step = pl.program_id(0)

    def x_copy(i):
        rows = pl.ds(pl.multiple_of(i * TQ, TQ), TQ)
        return pltpu.make_async_copy(x_hbm.at[rows, :], x_ref.at[rows, :], sems.at[i])

    wk_copy = pltpu.make_async_copy(wkt_hbm, wkt_ref, sems.at[NQB])
    wv_copy = pltpu.make_async_copy(wvt_hbm, wvt_ref, sems.at[NQB + 1])
    wq_copy = pltpu.make_async_copy(wq_hbm, wq_ref, sems.at[NQB + 2])
    late_copies = (pltpu.make_async_copy(wo_hbm, wo_ref, sems.at[NQB + 3]),
                   pltpu.make_async_copy(wg_hbm, wg_ref, sems.at[NQB + 4]),
                   pltpu.make_async_copy(wu_hbm, wu_ref, sems.at[NQB + 5]),
                   pltpu.make_async_copy(wd_hbm, wd_ref, sems.at[NQB + 6]),
                   pltpu.make_async_copy(gw_hbm, gw_ref, sems.at[NQB + 7]))

    def build_qb_rows(qb, g, rows):
        for r in rows:
            qb_ref[g, r] = jnp.broadcast_to(qf_ref[qb, g, pl.ds(r, 1), :], (8, TQ))

    def build_qb(qb):
        for g in range(NG):
            n = min(HPG, H - g * HPG) * DH
            build_qb_rows(qb, g, list(range(n)) + [BROW])

    @pl.when(step == 0)
    def _setup():
        wq_copy.start()
        wk_copy.start()
        wv_copy.start()
        for i in range(NQB):
            x_copy(i).start()

        wq_copy.wait()
        wt_ref[pl.ds(0, D // 2), :] = _pack(wq_ref[...].astype(F32).T.astype(BF16))
        wk_copy.wait()
        wv_copy.wait()
        zpad = jnp.zeros((VROWS - DH, D), F32)
        wkv = jnp.concatenate([wkt_ref[...].astype(F32), zpad,
                               wvt_ref[...].astype(F32), zpad], axis=0)
        wt_ref[pl.ds(D // 2, VROWS), :] = _pack(wkv.astype(BF16))

        def chunk(i, vmax, qb_groups):
            x_copy(i).wait()
            for g in qb_groups:
                build_qb_rows(0, g, range(BROW))
            rows = pl.ds(pl.multiple_of(i * TQ, TQ), TQ)
            lane = jax.lax.broadcasted_iota(jnp.int32, (TQ, 128), 1)
            vrow = jax.lax.broadcasted_iota(jnp.int32, (VROWS, TQ), 0)
            xi = x_ref[rows, :]
            kvt = jax.lax.dot_general(_unpack(wt_ref[pl.ds(D // 2, VROWS), :]), xi, NT,
                                      preferred_element_type=F32)
            kt = (kvt[:VROWS] * (DH ** -0.5 * LOG2E)).astype(BF16).astype(F32)
            km_ref[...] = jnp.maximum(km_ref[...], jnp.sum(kt * kt, axis=0, keepdims=True))
            krept = jnp.concatenate([kt[:DH]] * HPG + [jnp.zeros((128 - BROW, TQ), F32)], axis=0)
            kf_ref[...] = krept.T
            ev = kf_ref[pl.ds(0, TQ // 2, stride=2), :].reshape(TQ // 16, 1, 8, 128)
            od = kf_ref[pl.ds(1, TQ // 2, stride=2), :].reshape(TQ // 16, 1, 8, 128)
            kperm = jnp.concatenate([ev, od], axis=1).reshape(TQ, 128)
            for j in range(HPG):
                m = (lane >= j * DH) & (lane < (j + 1) * DH)
                kj = jnp.where(m, kperm, jnp.where(lane == BROW, 1.0, 0.0))
                kj = _pack(kj.astype(BF16))
                kpv_ref[j, pl.ds(pl.multiple_of(i * (NVB // 2), 8), NVB // 2), :] = (
                    jnp.concatenate([kj[c * CK // 2:(c * CK + NV_PAT[c]) // 2]
                                     for c in range(TQ // CK)], axis=0))
                kpm_ref[j, pl.ds(pl.multiple_of(i * (NMB // 2), 8), NMB // 2), :] = (
                    jnp.concatenate([kj[(c * CK + NV_PAT[c]) // 2:(c + 1) * CK // 2]
                                     for c in range(TQ // CK)], axis=0))
            kv = jnp.concatenate([kperm[c * CK:c * CK + NV_PAT[c]] for c in range(TQ // CK)],
                                 axis=0)
            for d in range(DH):
                kb_ref[d, pl.ds(pl.multiple_of(i * NVB, 16), NVB), :] = jnp.broadcast_to(
                    kv[:, d:d + 1], (NVB, 128))
            vt = kvt[VROWS:].astype(BF16).astype(F32)
            vmax = jnp.maximum(vmax, jnp.abs(vt))
            vt_ref[0, :, rows] = jnp.where(vrow == DH, 1.0, vt)
            vtb = jnp.concatenate([vt[DH:], vt[:DH]], axis=0)
            vt_ref[1, :, rows] = jnp.where(vrow == 0, 1.0, vtb)
            proj = jax.lax.dot_general(_unpack(wt_ref[pl.ds(0, D // 2), :]), xi, NT,
                                       preferred_element_type=F32)
            for g in range(NG):
                n = min(HPG, H - g * HPG) * DH
                qg = proj[g * BROW: g * BROW + n]
                n2_ref[g, :, rows] = jnp.sum(qg * qg, axis=0, keepdims=True)
                blk = jnp.concatenate([qg, jnp.zeros((128 - n, TQ), F32)], axis=0).astype(BF16)
                qt_ref[i, g] = _pack(blk)
                qf_ref[i, g] = blk.astype(F32)
            return vmax

        km_ref[...] = jnp.zeros((1, TQ), F32)
        carry = chunk(0, jnp.zeros((VROWS, TQ), F32), ())
        gpi = NG // (NQB - 1)
        vmax = jax.lax.fori_loop(
            1, NQB,
            lambda i, c: chunk(i, c, [(i - 1) * gpi + u for u in range(gpi)]), carry)
        for cp in late_copies:
            cp.start()
        k2 = jnp.max(km_ref[...])
        shifts = [jnp.sqrt(n2_ref[g] * k2) * 1.02 for g in range(NG)]
        cmax = shifts[0]
        for c in shifts[1:]:
            cmax = jnp.maximum(cmax, c)
        cm = jnp.max(cmax, axis=1, keepdims=True)
        vm = jnp.max(jnp.max(vmax, axis=0, keepdims=True), axis=1, keepdims=True)
        ok = jnp.logical_and(cm <= SHIFT_MAX, vm >= jnp.exp2(2.0 * cm - 100.0))
        safe = jnp.max(ok.astype(jnp.int32)) == 1
        flag_ref[0] = safe.astype(jnp.int32)
        for g in range(NG):
            c = jnp.where(safe, shifts[g], 0.0)
            crow = pltpu.pack_elementwise([-c, jnp.zeros_like(c)], packed_dtype=BF16)
            cf = (-c).astype(BF16).astype(F32)
            for i in range(NQB):
                qt_ref[i, g, pl.ds(BROW // 2, 1), :] = crow[:, i * TQ:(i + 1) * TQ]
                qf_ref[i, g, pl.ds(BROW, 1), :] = cf[:, i * TQ:(i + 1) * TQ]
            build_qb_rows(0, g, [BROW])

    q0 = pl.multiple_of(step * TQ, TQ)
    safe = flag_ref[0] == 1

    @pl.when(safe)
    def _fast():
        def produce(g, j, c, t):
            kc = _unpack(kpm_ref[j, pl.ds(MOFF[c] // 2, NMS[c] // 2), :])
            q = _unpack(qt_ref[step, g])
            p_ref[t % NBUF, pl.ds(0, NMS[c] // 2), :] = _pk16(
                jnp.exp2(jnp.dot(kc, q, preferred_element_type=F32)))

        def vpu_rows(g, j, r0):
            acc = qb_ref[g, BROW]
            for d in range(DH):
                kb = kb_ref[d, pl.ds(r0, 8), :]
                acc = acc + jnp.concatenate([kb] * (TQ // 128), axis=1) * qb_ref[g, j * DH + d]
            return jnp.exp2(acc)

        def produce_v(g, j, c, t):
            slot = t % NBV
            for b in range(NVS[c] // 16):
                e2 = vpu_rows(g, j, VOFF[c] + b * 16 + 8)
                e1 = vpu_rows(g, j, VOFF[c] + b * 16)
                pv_ref[slot, pl.ds(b * 8, 8), :] = pltpu.pack_elementwise([e1, e2],
                                                                          packed_dtype=BF16)

        def group(g, nheads, g_next):
            items = [(c, j) for c in range(NCK) for j in range(nheads)]
            n = len(items)
            for t, (c, j) in enumerate(items):
                for fn, la in ((produce, LA), (produce_v, LV)):
                    tn = t + la
                    if tn < n:
                        cn, jn = items[tn]
                        fn(g, jn, cn, tn)
                    elif g_next is not None:
                        fn(g_next, tn - n, 0, tn)
                p = jnp.concatenate([pv_ref[t % NBV, pl.ds(0, NVS[c] // 2), :],
                                     p_ref[t % NBUF, pl.ds(0, NMS[c] // 2), :]], axis=0)
                r = jnp.dot(vt_ref[j % 2, :, pl.ds(c * CK, CK)], _unpack(p),
                            preferred_element_type=F32)
                if c == 0:
                    acc_ref[j, pl.ds(0, VROWS), :] = r
                elif c < NCK - 1:
                    acc_ref[j, pl.ds(0, VROWS), :] = acc_ref[j, pl.ds(0, VROWS), :] + r
                else:
                    ot_ref[g * HPG + j] = acc_ref[j, pl.ds(0, VROWS), :] + r

        for c in range(LA):
            produce(0, c, 0, c)
        for c in range(LV):
            produce_v(0, c, 0, c)

        def body(g, carry):
            group(g, HPG, g + 1)
            return carry

        jax.lax.fori_loop(0, NG - 1, body, 0)
        group(NG - 1, H - (NG - 1) * HPG, None)

    @pl.when(jnp.logical_not(safe))
    def _slow():
        def body(it, carry):
            hp = it // (TQ // 128)
            cols = pl.ds(pl.multiple_of((it % (TQ // 128)) * 128, 128), 128)
            g = hp // (HPG // 2)
            jp = hp % (HPG // 2)
            q = _unpack(qt_ref[step, g, :, cols])
            nvk = VOFF[NCK]
            for par in range(2):
                j = 2 * jp + par
                s_ref[pl.ds(0, nvk), :] = jnp.dot(_unpack(kpv_ref[j]), q,
                                                  preferred_element_type=F32)
                s_ref[pl.ds(nvk, S - nvk), :] = jnp.dot(_unpack(kpm_ref[j]), q,
                                                        preferred_element_type=F32)
                m = jnp.max(s_ref[...], axis=0, keepdims=True)
                e = _pk16(jnp.exp2(s_ref[...] - m))
                pieces = []
                for c in range(NCK):
                    pieces += [e[VOFF[c] // 2:VOFF[c + 1] // 2],
                               e[(nvk + MOFF[c]) // 2:(nvk + MOFF[c + 1]) // 2]]
                p = _unpack(jnp.concatenate(pieces, axis=0))
                acc = jnp.dot(vt_ref[par], p, preferred_element_type=F32)
                ot_ref[2 * hp + par, :, cols] = acc
            return carry

        jax.lax.fori_loop(0, (H // 2) * (TQ // 128), body, 0)

    @pl.when(step == 0)
    def _wait_weights():
        for cp in late_copies:
            cp.wait()

    xb = x_ref[pl.ds(q0, TQ), :]
    b = jnp.zeros((TQ, D), F32)
    for f in range(FF // FC):
        gate = jnp.dot(xb, wg_ref[:, pl.ds(f * FC, FC)], preferred_element_type=F32)
        up = jnp.dot(xb, wu_ref[:, pl.ds(f * FC, FC)], preferred_element_type=F32)
        hh = (jnp.maximum(gate, 0.0) * up).astype(BF16)
        b = b + jnp.dot(hh, wd_ref[pl.ds(f * FC, FC), :], preferred_element_type=F32)

    build_qb(jnp.minimum(step + 1, NQB - 1))

    row = jax.lax.broadcasted_iota(jnp.int32, (8, TQ), 0)
    parts = []
    for hp in range(H // 2):
        a0 = ot_ref[2 * hp]
        a1 = ot_ref[2 * hp + 1]
        a0 = a0 * (1.0 / a0[DH:DH + 1, :])
        a1 = a1 * (1.0 / a1[0:1, :])
        parts += [a0[0:16], jnp.where(row < 4, a0[16:24], a1[0:8]), a1[8:24]]
    ot = jnp.concatenate(parts, axis=0).astype(BF16)
    a = jax.lax.dot_general(ot, wo_ref[...], TN, preferred_element_type=F32)

    gw = gw_ref[...].astype(F32)
    xf = xb.astype(F32)
    zp = xf[:, 0:128] * gw[0:1]
    for t in range(1, D // 128):
        zp = zp + xf[:, t * 128:(t + 1) * 128] * gw[t:t + 1]
    z = jnp.sum(zp, axis=-1, keepdims=True)
    g = 1.0 / (1.0 + jnp.exp(-z))
    o_ref[...] = (g * a + (1.0 - g) * b).astype(o_ref.dtype)


@jax.jit
def pallas_gated_mix__grouped_kv_mqa__glu_gated_reglu__prompt_kernel(
    A_x: jax.Array,
    A_wq: jax.Array,
    A_wk: jax.Array,
    A_wv: jax.Array,
    A_wo: jax.Array,
    B_x: jax.Array,
    B_W_gate: jax.Array,
    B_W_up: jax.Array,
    B_W_down: jax.Array,
    gate_w: jax.Array,
):
    x = A_x.reshape(S, D)
    gw = gate_w.reshape(D // 128, 128)

    out = pl.pallas_call(
        _kernel,
        grid=(NQB,),
        in_specs=[pl.BlockSpec(memory_space=pl.ANY)] * 9,
        out_specs=pl.BlockSpec((TQ, D), lambda i: (i, 0)),
        out_shape=jax.ShapeDtypeStruct((S, D), BF16),
        scratch_shapes=[
            pltpu.VMEM((S, D), BF16),
            pltpu.VMEM((D, D), BF16),
            pltpu.VMEM((D, D), BF16),
            pltpu.VMEM((D, FF), BF16),
            pltpu.VMEM((D, FF), BF16),
            pltpu.VMEM((FF, D), BF16),
            pltpu.VMEM((WROWS // 2 + 8, D), U32),
            pltpu.VMEM((TQ, 128), F32),
            pltpu.VMEM((HPG, MOFF[NCK] // 2, 128), U32),
            pltpu.VMEM((HPG, VOFF[NCK] // 2, 128), U32),
            pltpu.VMEM((DH, VOFF[NCK], 128), F32),
            pltpu.VMEM((2, VROWS, S), F32),
            pltpu.VMEM((NQB, NG, 64, TQ), U32),
            pltpu.VMEM((NQB, NG, 128, TQ), F32),
            pltpu.VMEM((NG, 128, 8, TQ), F32),
            pltpu.VMEM((NBUF, CK // 2, TQ), U32),
            pltpu.VMEM((NBV, 16, TQ), U32),
            pltpu.VMEM((S, 128), F32),
            pltpu.VMEM((H, VROWS, TQ), F32),
            pltpu.VMEM((HPG, VROWS + 8, TQ), F32),
            pltpu.VMEM((NG, 1, S), F32),
            pltpu.VMEM((DH, D), BF16),
            pltpu.VMEM((DH, D), BF16),
            pltpu.VMEM((D // 128, 128), BF16),
            pltpu.VMEM((1, TQ), F32),
            pltpu.SMEM((1,), jnp.int32),
            pltpu.SemaphoreType.DMA((NQB + 8,)),
        ],
        compiler_params=pltpu.CompilerParams(
            dimension_semantics=("arbitrary",),
            vmem_limit_bytes=100 * 1024 * 1024,
        ),
    )(x, A_wq, A_wk.T, A_wv.T, gw, A_wo, B_W_gate, B_W_up, B_W_down)
    return out.reshape(1, S, D)
```

```python
import jax
import jax.numpy as jnp
import jax.experimental.pallas as pl
import jax.experimental.pallas.tpu as pltpu

F32 = jnp.float32
BF16 = jnp.bfloat16
U32 = jnp.uint32

S = 2048
D = 640
H = 32
DH = 20
FF = 1536
HPG = 6
NG = 6
BROW = HPG * DH
VROWS = 24
TQ = 512
NQB = S // TQ
CK = 128
NCK = S // CK
LA = 2
NBUF = LA + 1
FC = 512
NV_PAT = (16, 16, 16, 16)
NVS = [NV_PAT[c % len(NV_PAT)] for c in range(NCK)]
NMS = [CK - v for v in NVS]
VOFF = [sum(NVS[:c]) for c in range(NCK + 1)]
MOFF = [sum(NMS[:c]) for c in range(NCK + 1)]
NVB = sum(NV_PAT)
NMB = TQ - NVB
LV = 1
NBV = LV + 1
WROWS = D + 2 * VROWS
LOG2E = 1.4426950408889634
SHIFT_MAX = 48.0

NT = (((1,), (1,)), ((), ()))
TN = (((0,), (0,)), ((), ()))


def _pack(x_bf16):
    return pltpu.bitcast(x_bf16, U32)


def _unpack(x_u32):
    return pltpu.bitcast(x_u32, BF16)


def _pk16(e):
    n, w = e.shape
    e4 = e.reshape(n // 16, 2, 8, w)
    return pltpu.pack_elementwise([e4[:, 0], e4[:, 1]], packed_dtype=BF16).reshape(n // 2, w)


def _kernel(x_hbm, wq_hbm, wkt_hbm, wvt_hbm, gw_hbm, wo_hbm, wg_hbm, wu_hbm, wd_hbm,
            o_ref,
            x_ref, wq_ref, wo_ref, wg_ref, wu_ref, wd_ref,
            wt_ref, kf_ref, kpm_ref, kpv_ref, kb_ref, vt_ref, qt_ref, qf_ref, qb_ref, p_ref, pv_ref,
            s_ref, ot_ref, acc_ref, n2_ref, wkt_ref, wvt_ref, gw_ref, km_ref, flag_ref, sems):
    step = pl.program_id(0)

    def x_copy(i):
        rows = pl.ds(pl.multiple_of(i * TQ, TQ), TQ)
        return pltpu.make_async_copy(x_hbm.at[rows, :], x_ref.at[rows, :], sems.at[i])

    wk_copy = pltpu.make_async_copy(wkt_hbm, wkt_ref, sems.at[NQB])
    wv_copy = pltpu.make_async_copy(wvt_hbm, wvt_ref, sems.at[NQB + 1])
    wq_copy = pltpu.make_async_copy(wq_hbm, wq_ref, sems.at[NQB + 2])
    late_copies = (pltpu.make_async_copy(wo_hbm, wo_ref, sems.at[NQB + 3]),
                   pltpu.make_async_copy(wg_hbm, wg_ref, sems.at[NQB + 4]),
                   pltpu.make_async_copy(wu_hbm, wu_ref, sems.at[NQB + 5]),
                   pltpu.make_async_copy(wd_hbm, wd_ref, sems.at[NQB + 6]),
                   pltpu.make_async_copy(gw_hbm, gw_ref, sems.at[NQB + 7]))

    def build_qb_rows(qb, g, rows):
        for r in rows:
            qb_ref[g, r] = jnp.broadcast_to(qf_ref[qb, g, pl.ds(r, 1), :], (8, TQ))

    def build_qb(qb):
        for g in range(NG):
            n = min(HPG, H - g * HPG) * DH
            build_qb_rows(qb, g, list(range(n)) + [BROW])

    @pl.when(step == 0)
    def _setup():
        wk_copy.start()
        wv_copy.start()
        x_copy(0).start()
        wq_copy.start()
        for i in range(1, NQB):
            x_copy(i).start()

        wk_copy.wait()
        wv_copy.wait()
        zpad = jnp.zeros((VROWS - DH, D), F32)
        wkv = jnp.concatenate([wkt_ref[...].astype(F32), zpad,
                               wvt_ref[...].astype(F32), zpad], axis=0)
        wt_ref[pl.ds(D // 2, VROWS), :] = _pack(wkv.astype(BF16))

        def chunk(i, vmax, qb_groups):
            x_copy(i).wait()
            for g in qb_groups:
                build_qb_rows(0, g, range(BROW))
            rows = pl.ds(pl.multiple_of(i * TQ, TQ), TQ)
            lane = jax.lax.broadcasted_iota(jnp.int32, (TQ, 128), 1)
            vrow = jax.lax.broadcasted_iota(jnp.int32, (VROWS, TQ), 0)
            xi = x_ref[rows, :]
            kvt = jax.lax.dot_general(_unpack(wt_ref[pl.ds(D // 2, VROWS), :]), xi, NT,
                                      preferred_element_type=F32)
            kt = (kvt[:VROWS] * (DH ** -0.5 * LOG2E)).astype(BF16).astype(F32)
            km_ref[...] = jnp.maximum(km_ref[...], jnp.sum(kt * kt, axis=0, keepdims=True))
            krept = jnp.concatenate([kt[:DH]] * HPG + [jnp.zeros((128 - BROW, TQ), F32)], axis=0)
            kf_ref[...] = krept.T
            ev = kf_ref[pl.ds(0, TQ // 2, stride=2), :].reshape(TQ // 16, 1, 8, 128)
            od = kf_ref[pl.ds(1, TQ // 2, stride=2), :].reshape(TQ // 16, 1, 8, 128)
            kperm = jnp.concatenate([ev, od], axis=1).reshape(TQ, 128)
            for j in range(HPG):
                m = (lane >= j * DH) & (lane < (j + 1) * DH)
                kj = jnp.where(m, kperm, jnp.where(lane == BROW, 1.0, 0.0))
                kj = _pack(kj.astype(BF16))
                kpv_ref[j, pl.ds(pl.multiple_of(i * (NVB // 2), 8), NVB // 2), :] = (
                    jnp.concatenate([kj[c * CK // 2:(c * CK + NV_PAT[c]) // 2]
                                     for c in range(TQ // CK)], axis=0))
                kpm_ref[j, pl.ds(pl.multiple_of(i * (NMB // 2), 8), NMB // 2), :] = (
                    jnp.concatenate([kj[(c * CK + NV_PAT[c]) // 2:(c + 1) * CK // 2]
                                     for c in range(TQ // CK)], axis=0))
            kv = jnp.concatenate([kperm[c * CK:c * CK + NV_PAT[c]] for c in range(TQ // CK)],
                                 axis=0)
            for d in range(DH):
                kb_ref[d, pl.ds(pl.multiple_of(i * NVB, 16), NVB), :] = jnp.broadcast_to(
                    kv[:, d:d + 1], (NVB, 128))
            vt = kvt[VROWS:].astype(BF16).astype(F32)
            vmax = jnp.maximum(vmax, jnp.abs(vt))
            vt_ref[0, :, rows] = jnp.where(vrow == DH, 1.0, vt)
            vtb = jnp.concatenate([vt[DH:], vt[:DH]], axis=0)
            vt_ref[1, :, rows] = jnp.where(vrow == 0, 1.0, vtb)
            if isinstance(i, int) and i == 0:
                wq_copy.wait()
                wt_ref[pl.ds(0, D // 2), :] = _pack(wq_ref[...].astype(F32).T.astype(BF16))
            proj = jax.lax.dot_general(_unpack(wt_ref[pl.ds(0, D // 2), :]), xi, NT,
                                       preferred_element_type=F32)
            for g in range(NG):
                n = min(HPG, H - g * HPG) * DH
                qg = proj[g * BROW: g * BROW + n]
                n2_ref[g, :, rows] = jnp.sum(qg * qg, axis=0, keepdims=True)
                blk = jnp.concatenate([qg, jnp.zeros((128 - n, TQ), F32)], axis=0).astype(BF16)
                qt_ref[i, g] = _pack(blk)
                qf_ref[i, g] = blk.astype(F32)
            return vmax

        km_ref[...] = jnp.zeros((1, TQ), F32)
        carry = chunk(0, jnp.zeros((VROWS, TQ), F32), ())
        gpi = NG // (NQB - 1)
        vmax = jax.lax.fori_loop(
            1, NQB,
            lambda i, c: chunk(i, c, [(i - 1) * gpi + u for u in range(gpi)]), carry)
        for cp in late_copies:
            cp.start()
        k2 = jnp.max(km_ref[...])
        shifts = [jnp.sqrt(n2_ref[g] * k2) * 1.02 for g in range(NG)]
        cmax = shifts[0]
        for c in shifts[1:]:
            cmax = jnp.maximum(cmax, c)
        cm = jnp.max(cmax, axis=1, keepdims=True)
        vm = jnp.max(jnp.max(vmax, axis=0, keepdims=True), axis=1, keepdims=True)
        ok = jnp.logical_and(cm <= SHIFT_MAX, vm >= jnp.exp2(2.0 * cm - 100.0))
        safe = jnp.max(ok.astype(jnp.int32)) == 1
        flag_ref[0] = safe.astype(jnp.int32)
        for g in range(NG):
            c = jnp.where(safe, shifts[g], 0.0)
            crow = pltpu.pack_elementwise([-c, jnp.zeros_like(c)], packed_dtype=BF16)
            cf = (-c).astype(BF16).astype(F32)
            for i in range(NQB):
                qt_ref[i, g, pl.ds(BROW // 2, 1), :] = crow[:, i * TQ:(i + 1) * TQ]
                qf_ref[i, g, pl.ds(BROW, 1), :] = cf[:, i * TQ:(i + 1) * TQ]
            build_qb_rows(0, g, [BROW])

    q0 = pl.multiple_of(step * TQ, TQ)
    safe = flag_ref[0] == 1

    @pl.when(safe)
    def _fast():
        def produce(g, j, c, t):
            kc = _unpack(kpm_ref[j, pl.ds(MOFF[c] // 2, NMS[c] // 2), :])
            q = _unpack(qt_ref[step, g])
            p_ref[t % NBUF, pl.ds(0, NMS[c] // 2), :] = _pk16(
                jnp.exp2(jnp.dot(kc, q, preferred_element_type=F32)))

        def vpu_rows(g, j, r0):
            acc = qb_ref[g, BROW]
            for d in range(DH):
                kb = kb_ref[d, pl.ds(r0, 8), :]
                acc = acc + jnp.concatenate([kb] * (TQ // 128), axis=1) * qb_ref[g, j * DH + d]
            return jnp.exp2(acc)

        def produce_v(g, j, c, t):
            slot = t % NBV
            for b in range(NVS[c] // 16):
                e2 = vpu_rows(g, j, VOFF[c] + b * 16 + 8)
                e1 = vpu_rows(g, j, VOFF[c] + b * 16)
                pv_ref[slot, pl.ds(b * 8, 8), :] = pltpu.pack_elementwise([e1, e2],
                                                                          packed_dtype=BF16)

        def group(g, nheads, g_next):
            items = [(c, j) for c in range(NCK) for j in range(nheads)]
            n = len(items)
            for t, (c, j) in enumerate(items):
                for fn, la in ((produce, LA), (produce_v, LV)):
                    tn = t + la
                    if tn < n:
                        cn, jn = items[tn]
                        fn(g, jn, cn, tn)
                    elif g_next is not None:
                        fn(g_next, tn - n, 0, tn)
                p = jnp.concatenate([pv_ref[t % NBV, pl.ds(0, NVS[c] // 2), :],
                                     p_ref[t % NBUF, pl.ds(0, NMS[c] // 2), :]], axis=0)
                r = jnp.dot(vt_ref[j % 2, :, pl.ds(c * CK, CK)], _unpack(p),
                            preferred_element_type=F32)
                if c == 0:
                    acc_ref[j, pl.ds(0, VROWS), :] = r
                elif c < NCK - 1:
                    acc_ref[j, pl.ds(0, VROWS), :] = acc_ref[j, pl.ds(0, VROWS), :] + r
                else:
                    ot_ref[g * HPG + j] = acc_ref[j, pl.ds(0, VROWS), :] + r

        for c in range(LA):
            produce(0, c, 0, c)
        for c in range(LV):
            produce_v(0, c, 0, c)

        def body(g, carry):
            group(g, HPG, g + 1)
            return carry

        jax.lax.fori_loop(0, NG - 1, body, 0)
        group(NG - 1, H - (NG - 1) * HPG, None)

    @pl.when(jnp.logical_not(safe))
    def _slow():
        def body(it, carry):
            hp = it // (TQ // 128)
            cols = pl.ds(pl.multiple_of((it % (TQ // 128)) * 128, 128), 128)
            g = hp // (HPG // 2)
            jp = hp % (HPG // 2)
            q = _unpack(qt_ref[step, g, :, cols])
            nvk = VOFF[NCK]
            for par in range(2):
                j = 2 * jp + par
                s_ref[pl.ds(0, nvk), :] = jnp.dot(_unpack(kpv_ref[j]), q,
                                                  preferred_element_type=F32)
                s_ref[pl.ds(nvk, S - nvk), :] = jnp.dot(_unpack(kpm_ref[j]), q,
                                                        preferred_element_type=F32)
                m = jnp.max(s_ref[...], axis=0, keepdims=True)
                e = _pk16(jnp.exp2(s_ref[...] - m))
                pieces = []
                for c in range(NCK):
                    pieces += [e[VOFF[c] // 2:VOFF[c + 1] // 2],
                               e[(nvk + MOFF[c]) // 2:(nvk + MOFF[c + 1]) // 2]]
                p = _unpack(jnp.concatenate(pieces, axis=0))
                acc = jnp.dot(vt_ref[par], p, preferred_element_type=F32)
                ot_ref[2 * hp + par, :, cols] = acc
            return carry

        jax.lax.fori_loop(0, (H // 2) * (TQ // 128), body, 0)

    @pl.when(step == 0)
    def _wait_weights():
        for cp in late_copies:
            cp.wait()

    xb = x_ref[pl.ds(q0, TQ), :]
    b = jnp.zeros((TQ, D), F32)
    for f in range(FF // FC):
        gate = jnp.dot(xb, wg_ref[:, pl.ds(f * FC, FC)], preferred_element_type=F32)
        up = jnp.dot(xb, wu_ref[:, pl.ds(f * FC, FC)], preferred_element_type=F32)
        hh = (jnp.maximum(gate, 0.0) * up).astype(BF16)
        b = b + jnp.dot(hh, wd_ref[pl.ds(f * FC, FC), :], preferred_element_type=F32)

    build_qb(jnp.minimum(step + 1, NQB - 1))

    row = jax.lax.broadcasted_iota(jnp.int32, (8, TQ), 0)
    parts = []
    for hp in range(H // 2):
        a0 = ot_ref[2 * hp]
        a1 = ot_ref[2 * hp + 1]
        a0 = a0 * (1.0 / a0[DH:DH + 1, :])
        a1 = a1 * (1.0 / a1[0:1, :])
        parts += [a0[0:16], jnp.where(row < 4, a0[16:24], a1[0:8]), a1[8:24]]
    ot = jnp.concatenate(parts, axis=0).astype(BF16)
    a = jax.lax.dot_general(ot, wo_ref[...], TN, preferred_element_type=F32)

    gw = gw_ref[...].astype(F32)
    xf = xb.astype(F32)
    zp = xf[:, 0:128] * gw[0:1]
    for t in range(1, D // 128):
        zp = zp + xf[:, t * 128:(t + 1) * 128] * gw[t:t + 1]
    z = jnp.sum(zp, axis=-1, keepdims=True)
    g = 1.0 / (1.0 + jnp.exp(-z))
    o_ref[...] = (g * a + (1.0 - g) * b).astype(o_ref.dtype)


@jax.jit
def pallas_gated_mix__grouped_kv_mqa__glu_gated_reglu__prompt_kernel(
    A_x: jax.Array,
    A_wq: jax.Array,
    A_wk: jax.Array,
    A_wv: jax.Array,
    A_wo: jax.Array,
    B_x: jax.Array,
    B_W_gate: jax.Array,
    B_W_up: jax.Array,
    B_W_down: jax.Array,
    gate_w: jax.Array,
):
    x = A_x.reshape(S, D)
    gw = gate_w.reshape(D // 128, 128)

    out = pl.pallas_call(
        _kernel,
        grid=(NQB,),
        in_specs=[pl.BlockSpec(memory_space=pl.ANY)] * 9,
        out_specs=pl.BlockSpec((TQ, D), lambda i: (i, 0)),
        out_shape=jax.ShapeDtypeStruct((S, D), BF16),
        scratch_shapes=[
            pltpu.VMEM((S, D), BF16),
            pltpu.VMEM((D, D), BF16),
            pltpu.VMEM((D, D), BF16),
            pltpu.VMEM((D, FF), BF16),
            pltpu.VMEM((D, FF), BF16),
            pltpu.VMEM((FF, D), BF16),
            pltpu.VMEM((WROWS // 2 + 8, D), U32),
            pltpu.VMEM((TQ, 128), F32),
            pltpu.VMEM((HPG, MOFF[NCK] // 2, 128), U32),
            pltpu.VMEM((HPG, VOFF[NCK] // 2, 128), U32),
            pltpu.VMEM((DH, VOFF[NCK], 128), F32),
            pltpu.VMEM((2, VROWS, S), F32),
            pltpu.VMEM((NQB, NG, 64, TQ), U32),
            pltpu.VMEM((NQB, NG, 128, TQ), F32),
            pltpu.VMEM((NG, 128, 8, TQ), F32),
            pltpu.VMEM((NBUF, CK // 2, TQ), U32),
            pltpu.VMEM((NBV, 16, TQ), U32),
            pltpu.VMEM((S, 128), F32),
            pltpu.VMEM((H, VROWS, TQ), F32),
            pltpu.VMEM((HPG, VROWS + 8, TQ), F32),
            pltpu.VMEM((NG, 1, S), F32),
            pltpu.VMEM((DH, D), BF16),
            pltpu.VMEM((DH, D), BF16),
            pltpu.VMEM((D // 128, 128), BF16),
            pltpu.VMEM((1, TQ), F32),
            pltpu.SMEM((1,), jnp.int32),
            pltpu.SemaphoreType.DMA((NQB + 8,)),
        ],
        compiler_params=pltpu.CompilerParams(
            dimension_semantics=("arbitrary",),
            vmem_limit_bytes=100 * 1024 * 1024,
        ),
    )(x, A_wq, A_wk.T, A_wv.T, gw, A_wo, B_W_gate, B_W_up, B_W_down)
    return out.reshape(1, S, D)
```
